```python
import jax
import jax.numpy as jnp

def _softmax(x, axis=-1):
    return jax.nn.softmax(x, axis=axis)
def _gelu(x):
    return jax.nn.gelu(x, approximate=True)
def _silu(x):
    return jax.nn.silu(x)
def _sigmoid(x):
    return jax.nn.sigmoid(x)
def _layernorm(x, axis=-1, eps=1e-5):
    m = jnp.mean(x, axis=axis, keepdims=True)
    v = jnp.var(x, axis=axis, keepdims=True)
    return (x - m) / jnp.sqrt(v + eps)
def _scatter_add(tgt, idx, src, axis=0):
    return tgt.at[idx].add(src)
def _segment_sum(src, seg, n):
    return jax.ops.segment_sum(src, seg, n)
class _Rng:
    def __init__(self, key):
        self._k = key
    def _next(self):
        self._k, sub = jax.random.split(self._k)
        return sub
    def normal(self, shape):
        return jax.random.normal(self._next(), shape, dtype=jnp.bfloat16)
    def randint(self, lo, hi, shape):
        return jax.random.randint(self._next(), shape, lo, hi, dtype=jnp.int32)
    def uniform(self, shape, lo=0.0, hi=1.0):
        return jax.random.uniform(self._next(), shape, jnp.bfloat16, lo, hi)
    def permutation(self, n):
        return jax.random.permutation(self._next(), n)


kernel_name = 'gated_mix__mha_block_cached__compressed_kv_cla__decode'

def setup_inputs():
    _rng = _Rng(jax.random.key(int.from_bytes(__import__("os").urandom(4), "little")))
    _w = (lambda a: (lambda t: t.astype(jnp.bfloat16) if jnp.issubdtype(t.dtype, jnp.floating) else t)(jnp.asarray(a)))
    def _A_setup():
        B, Sq, D = 2, 1, 512
        H, Sk, Dh = 32, 8192, 128
        return {
            "x": _w((lambda *s: _rng.normal(s) * 0.05)(B, Sq, D)),
            "k_cache": _w((lambda *s: _rng.normal(s) * 0.05)(B, H, Sk, Dh)),
            "v_cache": _w((lambda *s: _rng.normal(s) * 0.05)(B, H, Sk, Dh)),
            "wq": _w((lambda *s: _rng.normal(s) * 0.05)(D, H * Dh) * (D ** -0.5)),
            "wo": _w((lambda *s: _rng.normal(s) * 0.05)(H * Dh, D) * ((H * Dh) ** -0.5)),
        }
    _A_in = _A_setup()

    def _B_setup():
        B, H, Sq, Sk, D, M = 2, 32, 1, 8192, 128, 512
        Dc = 4 * D
        return {
            "x": _w((lambda *s: _rng.normal(s) * 0.05)(B, Sq, M)),
            "c_kv": _w((lambda *s: _rng.normal(s) * 0.05)(B, Sk, Dc)),
            "w_q": _w((lambda *s: _rng.normal(s) * 0.05)(M, H, D) * (M ** -0.5)),
            "w_uk": _w((lambda *s: _rng.normal(s) * 0.05)(Dc, H, D) * (Dc ** -0.5)),
            "w_uv": _w((lambda *s: _rng.normal(s) * 0.05)(Dc, H, D) * (Dc ** -0.5)),
            "w_o": _w((lambda *s: _rng.normal(s) * 0.05)(H, D, M) * ((H * D) ** -0.5)),
        }
    _B_in = _B_setup()

    return {
        "A_x": _A_in["x"],
        "A_k_cache": _A_in["k_cache"],
        "A_v_cache": _A_in["v_cache"],
        "A_wq": _A_in["wq"],
        "A_wo": _A_in["wo"],
        "B_x": _B_in["x"],
        "B_c_kv": _B_in["c_kv"],
        "B_w_q": _B_in["w_q"],
        "B_w_uk": _B_in["w_uk"],
        "B_w_uv": _B_in["w_uv"],
        "B_w_o": _B_in["w_o"],
        "gate_w": _w((lambda *s: _rng.normal(s) * 0.05)(512)),
    }

def reference(A_x, A_k_cache, A_v_cache, A_wq, A_wo, B_x, B_c_kv, B_w_q, B_w_uk, B_w_uv, B_w_o, gate_w):
    def _A_ref(x, k_cache, v_cache, wq, wo):
        B, Sq, D = x.shape
        H, Dh = 32, 128
        q = (lambda x, *d: x.transpose(*d))((x @ wq).reshape(B, Sq, H, Dh), 0, 2, 1, 3)
        scores = jnp.einsum("bhqd,bhkd->bhqk", q, k_cache) * (Dh ** -0.5)
        p = _softmax(scores, axis=-1)
        o = jnp.einsum("bhqk,bhkd->bhqd", p, v_cache)
        return (lambda x, *d: x.transpose(*d))(o, 0, 2, 1, 3).reshape(B, Sq, H * Dh) @ wo

    def _B_ref(x, c_kv, w_q, w_uk, w_uv, w_o):
        B, Sq, M = x.shape[0], x.shape[1], x.shape[2]
        Sk = c_kv.shape[1]
        H, D = w_q.shape[1], w_q.shape[2]
        q = jnp.einsum("bqm,mhd->bhqd", x, w_q)
        k = jnp.einsum("bkc,chd->bhkd", c_kv, w_uk)
        v = jnp.einsum("bkc,chd->bhkd", c_kv, w_uv)
        scores = jnp.einsum("bhqd,bhkd->bhqk", q, k) * (D ** -0.5)
        off = Sk - Sq
        qi = jnp.arange(Sq)[:, None]
        kj = jnp.arange(Sk)[None, :]
        cmask = kj <= (qi + off)
        scores = jnp.where(cmask[None, None], scores, -1e9)
        p = _softmax(scores, axis=-1)
        ctx = jnp.einsum("bhqk,bhkd->bhqd", p, v)
        return jnp.einsum("bhqd,hdm->bqm", ctx, w_o)

    x = A_x
    g = _sigmoid((x * gate_w).sum(-1, keepdims=True))
    a = _A_ref(x, A_k_cache, A_v_cache, A_wq, A_wo)
    b = _B_ref(x, B_c_kv, B_w_q, B_w_uk, B_w_uv, B_w_o)
    return g * a + (1 - g) * b
```

```python
import jax
import jax.numpy as jnp
from jax import lax
import jax.experimental.pallas as pl
import jax.experimental.pallas.tpu as pltpu

NB = 2
NH = 32
SK = 8192
DH = 128
DM = 512
NBH = NB * NH
TR = 128
G = 4
NTILE = 64

F32 = jnp.float32
BF16 = jnp.bfloat16
NT_DIMS = (((1,), (1,)), ((), ()))


def _tile_order(i):
    return (i % 4) * 16 + i // 4


def _kernel(x_hbm, gate_hbm, k_hbm, v_hbm, wq_hbm, wo_hbm, ckv_hbm, bwq_hbm, wuk_hbm,
            wuv_hbm, bwo_hbm, o_ref,
            x_v, gate_v, kbuf, vbuf, wq_v, wo_v, ckv_v, bwq_v, wuk_v, wuv_v, bwo_v,
            qa_s, oa_s, qabs_s, s_s, m_s, l_s, acc_s, outb_s,
            ksem, vsem, wsem, wosem):
    scale = DH ** -0.5

    def kv_tile(src, dst, sem, item, slot, t):
        t0 = pl.multiple_of(t * TR, TR)
        return pltpu.make_async_copy(
            src.at[pl.ds(pl.multiple_of(item * SK + t0, TR), TR)],
            dst.at[slot, pl.ds(t0, TR)], sem.at[slot])

    def issue_kv(item, slot):
        def body(i, c):
            t = _tile_order(i)
            kv_tile(k_hbm, kbuf, ksem, item, slot, t).start(priority=0)
            kv_tile(v_hbm, vbuf, vsem, item, slot, t).start(priority=1)
            return c
        lax.fori_loop(0, NTILE, body, 0, unroll=4)

    def rows_tile(src, dst, sem, rows, base, t):
        r0 = pl.multiple_of(base + t * rows, rows)
        return pltpu.make_async_copy(src.at[pl.ds(r0, rows)], dst.at[pl.ds(r0, rows)], sem)

    def issue_rows_pair(src0, dst0, base0, src1, dst1, base1, rows, sem):
        def body(i, c):
            t = _tile_order(i)
            rows_tile(src0, dst0, sem, rows, base0, t).start(priority=0)
            rows_tile(src1, dst1, sem, rows, base1, t).start(priority=1)
            return c
        lax.fori_loop(0, NTILE, body, 0, unroll=4)

    def issue_whole(src, dst, rows, sem):
        half = NTILE * rows
        issue_rows_pair(src, dst, 0, src, dst, half, rows, sem)

    def issue_wq():
        def tile(half, t):
            r0 = pl.multiple_of(half * 256 + (t // 4) * 16, 16)
            c0 = pl.multiple_of((t % 4) * 1024, 1024)
            return pltpu.make_async_copy(
                wq_hbm.at[pl.ds(r0, 16), pl.ds(c0, 1024)],
                wq_v.at[pl.ds(r0, 16), pl.ds(c0, 1024)], wsem.at[0])

        def body(i, c):
            t = _tile_order(i)
            tile(0, t).start(priority=0)
            tile(1, t).start(priority=1)
            return c
        lax.fori_loop(0, NTILE, body, 0, unroll=4)

    def wo_tile(half, i):
        t = _tile_order(i)
        r0 = half * 2048 + t * 32
        return pltpu.make_async_copy(wo_hbm.at[pl.ds(r0, 32)], wo_v.at[pl.ds(r0, 32)],
                                     wosem.at[i // 16])

    def wait_full(buf, sem):
        pltpu.make_async_copy(buf, buf, sem).wait()

    x_cp = pltpu.make_async_copy(x_hbm, x_v, wsem.at[10])
    g_cp = pltpu.make_async_copy(gate_hbm, gate_v, wsem.at[11])
    x_cp.start()
    g_cp.start()
    issue_wq()
    for s0 in range(G - 1):
        issue_kv(s0, s0)

    outb_s[...] = jnp.zeros_like(outb_s)

    x_cp.wait()
    g_cp.wait()
    x2 = x_v[...].astype(F32)
    xf = jnp.concatenate([jnp.broadcast_to(x2[0:1], (8, DM)),
                          jnp.broadcast_to(x2[1:2], (8, DM))], axis=0)
    xb = xf.astype(BF16)
    gate = gate_v[...].astype(F32).reshape(1, DM)
    g = jax.nn.sigmoid(jnp.sum(xf * gate, axis=-1, keepdims=True))

    wait_full(wq_v, wsem.at[0])
    qa = jnp.dot(xb, wq_v[...], preferred_element_type=F32).astype(BF16)
    qa_s[0] = jnp.concatenate([qa[0:8], qa[0:8]], axis=0)
    qa_s[1] = jnp.concatenate([qa[8:16], qa[8:16]], axis=0)

    def deinterleave(w_v, j):
        u = w_v.bitcast(jnp.uint32)[pl.ds(j, DM, stride=NH // 2), :]
        lo = pltpu.bitcast(u << 16, F32).astype(BF16)
        hi = pltpu.bitcast(u & jnp.uint32(0xFFFF0000), F32).astype(BF16)
        return lo, hi

    def b_prologue_group(grp):
        row = lax.broadcasted_iota(jnp.int32, (16, DH), 0) % 8
        tot = None
        for j in range(4 * grp, 4 * grp + 4):
            wq_pair = deinterleave(bwq_v, j)
            wk_pair = deinterleave(wuk_v, j)
            for e in range(2):
                r = (2 * j + e) % 8
                q = jnp.dot(xb, wq_pair[e], preferred_element_type=F32).astype(BF16)
                q = jnp.where(row == r, q, jnp.zeros_like(q))
                qabs = lax.dot_general(q, wk_pair[e], NT_DIMS, preferred_element_type=F32)
                tot = qabs if tot is None else tot + qabs
        qabs_s[0, 8 * grp:8 * grp + 8, :] = tot[0:8]
        qabs_s[1, 8 * grp:8 * grp + 8, :] = tot[8:16]

    CK = 2048

    def b_scores_chunk(b, j):
        q = qabs_s[b].astype(BF16)
        r0 = pl.multiple_of(b * SK + j * CK, CK)
        c = ckv_v[pl.ds(r0, CK), :]
        s = lax.dot_general(q, c, NT_DIMS, preferred_element_type=F32)
        s_s[b, :, pl.ds(pl.multiple_of(j * CK, CK), CK)] = s
        mx = jnp.max(s, axis=-1, keepdims=True)
        mx = jnp.broadcast_to(mx, (NH, 128))

        @pl.when(j == 0)
        def _():
            m_s[b] = mx

        @pl.when(j > 0)
        def _():
            m_s[b] = jnp.maximum(m_s[b], mx)

    def b_pv_chunk(b, j):
        r0 = pl.multiple_of(b * SK + j * CK, CK)
        c = ckv_v[pl.ds(r0, CK), :]
        s = s_s[b, :, pl.ds(pl.multiple_of(j * CK, CK), CK)]
        m = m_s[b][:, 0:1]
        p = jnp.exp((s - m) * scale)
        ls = jnp.broadcast_to(jnp.sum(p, axis=-1, keepdims=True), (NH, 128))
        pv = jnp.dot(p.astype(BF16), c, preferred_element_type=F32)

        @pl.when(j == 0)
        def _():
            l_s[b] = ls
            acc_s[b] = pv

        @pl.when(j > 0)
        def _():
            l_s[b] = l_s[b] + ls
            acc_s[b] = acc_s[b] + pv

    def b_normalize():
        for b in range(NB):
            acc_s[b] = acc_s[b] / l_s[b][:, 0:1]

    def b_epilogue_group(grp):
        row = lax.broadcasted_iota(jnp.int32, (16, DH), 0) % 8
        lhs = jnp.concatenate([acc_s[0, 8 * grp:8 * grp + 8, :], acc_s[1, 8 * grp:8 * grp + 8, :]],
                              axis=0).astype(BF16)
        tot = None
        for j in range(4 * grp, 4 * grp + 4):
            wv_pair = deinterleave(wuv_v, j)
            for e in range(2):
                h = 2 * j + e
                ctx = jnp.dot(lhs, wv_pair[e], preferred_element_type=F32).astype(BF16)
                ctx = jnp.where(row == h % 8, ctx, jnp.zeros_like(ctx))
                part = jnp.dot(ctx, bwo_v[h * DH:(h + 1) * DH, :], preferred_element_type=F32)
                tot = part if tot is None else tot + part
        outb_s[...] += tot

    def a_step(s):
        b = s // NH
        h = s % NH
        slot = s % G
        c0 = pl.multiple_of(h * DH, DH)
        q = qa_s[b, :, pl.ds(c0, DH)]
        wait_full(kbuf.at[slot], ksem.at[slot])
        sc = lax.dot_general(q, kbuf[slot], NT_DIMS, preferred_element_type=F32)
        m = jnp.max(sc, axis=-1, keepdims=True)
        p = jnp.exp((sc - m) * scale)
        l = jnp.sum(p, axis=-1, keepdims=True)
        wait_full(vbuf.at[slot], vsem.at[slot])
        o = jnp.dot(p.astype(BF16), vbuf[slot], preferred_element_type=F32)
        o = o / l
        oa_s[b, :, pl.ds(c0, DH)] = o[0:8, :]

    S_BWQ, S_WUK, S_CKV0, S_WUV, S_BWO = 0, 1, 2, 6, 7
    S_BPRO = 5
    S_BSC = S_BPRO + 4
    S_BPV = S_BSC + 8
    S_BEPI = S_BPV + 8
    N_LAST = NBH - (G - 1)

    def step(s, carry):
        nxt = s + (G - 1)

        @pl.when(nxt < NBH)
        def _():
            issue_kv(nxt, nxt % G)

        @pl.when(s == S_BWQ)
        def _():
            issue_whole(bwq_hbm, bwq_v, TR, wsem.at[1])

        @pl.when(s == S_WUK)
        def _():
            issue_whole(wuk_hbm, wuk_v, TR, wsem.at[2])

        @pl.when(jnp.logical_and(s >= S_CKV0, s < S_CKV0 + 4))
        def _():
            j = s - S_CKV0
            base = pl.multiple_of(j * 2048, 2048)
            issue_rows_pair(ckv_hbm, ckv_v, base, ckv_hbm, ckv_v, SK + base, 32, wsem.at[3])

        @pl.when(s == S_WUV)
        def _():
            issue_whole(wuv_hbm, wuv_v, TR, wsem.at[4])

        @pl.when(s == S_BWO)
        def _():
            issue_whole(bwo_hbm, bwo_v, 32, wsem.at[5])

        @pl.when(s == N_LAST - 1)
        def _():
            def body(i, c):
                wo_tile(0, i).start(priority=0)
                wo_tile(1, i).start(priority=1)
                return c
            lax.fori_loop(0, NTILE, body, 0, unroll=4)

        @pl.when(s == S_BPRO)
        def _():
            wait_full(bwq_v, wsem.at[1])
            wait_full(wuk_v, wsem.at[2])

        for grp in range(4):
            pl.when(s == S_BPRO + grp)(lambda grp=grp: b_prologue_group(grp))

        @pl.when(s == S_BSC)
        def _():
            wait_full(ckv_v, wsem.at[3])

        @pl.when(jnp.logical_and(s >= S_BSC, s < S_BSC + 8))
        def _():
            i = s - S_BSC
            b_scores_chunk(i // 4, i % 4)

        @pl.when(jnp.logical_and(s >= S_BPV, s < S_BPV + 8))
        def _():
            i = s - S_BPV
            b_pv_chunk(i // 4, i % 4)

        @pl.when(s == S_BEPI)
        def _():
            wait_full(wuv_v, wsem.at[4])
            wait_full(bwo_v, wsem.at[5])
            b_normalize()

        for grp in range(4):
            pl.when(s == S_BEPI + grp)(lambda grp=grp: b_epilogue_group(grp))

        a_step(s)
        return carry

    lax.fori_loop(0, NBH, step, 0)

    oa = jnp.concatenate([oa_s[0], oa_s[1]], axis=0).astype(BF16)
    acc = jnp.zeros((16, DM), F32)
    for jq in range(4):
        for i in range(16 * jq, 16 * jq + 16):
            wo_tile(0, i).wait()
            wo_tile(1, i).wait()
        for half in range(2):
            for st in range(4):
                hd = half * 16 + st * 4 + jq
                acc = acc + jnp.dot(oa[:, hd * DH:(hd + 1) * DH],
                                    wo_v[hd * DH:(hd + 1) * DH, :],
                                    preferred_element_type=F32)
    a_out = acc.astype(BF16).astype(F32)
    ob = outb_s[...]
    b0 = jnp.sum(ob[0:8], axis=0, keepdims=True).astype(BF16).astype(F32)
    b1 = jnp.sum(ob[8:16], axis=0, keepdims=True).astype(BF16).astype(F32)
    g0 = g[0:1, :]
    g1 = g[8:9, :]
    r0 = g0 * a_out[0:1, :] + (1.0 - g0) * b0
    r1 = g1 * a_out[8:9, :] + (1.0 - g1) * b1
    o_ref[...] = jnp.concatenate([r0, r1], axis=0).astype(o_ref.dtype)


@jax.jit
def pallas_gated_mix__mha_block_cached__compressed_kv_cla__decode_kernel(
    A_x: jax.Array,
    A_k_cache: jax.Array,
    A_v_cache: jax.Array,
    A_wq: jax.Array,
    A_wo: jax.Array,
    B_x: jax.Array,
    B_c_kv: jax.Array,
    B_w_q: jax.Array,
    B_w_uk: jax.Array,
    B_w_uv: jax.Array,
    B_w_o: jax.Array,
    gate_w: jax.Array,
):
    del B_x
    k2 = A_k_cache.reshape(NBH * SK, DH)
    v2 = A_v_cache.reshape(NBH * SK, DH)
    ckv2 = B_c_kv.reshape(NB * SK, DM)
    bwq2 = B_w_q.reshape(DM * NH, DH)
    wuk2 = B_w_uk.reshape(DM * NH, DH)
    wuv2 = B_w_uv.reshape(DM * NH, DH)
    bwo2 = B_w_o.reshape(NH * DH, DM)

    any_spec = pl.BlockSpec(memory_space=pl.ANY)
    scratch = [
        pltpu.VMEM((NB, DM), BF16),
        pltpu.VMEM((DM,), BF16),
        pltpu.VMEM((G, SK, DH), BF16),
        pltpu.VMEM((G, SK, DH), BF16),
        pltpu.VMEM((DM, NH * DH), BF16),
        pltpu.VMEM((NH * DH, DM), BF16),
        pltpu.VMEM((NB * SK, DM), BF16),
        pltpu.VMEM((DM * NH, DH), BF16),
        pltpu.VMEM((DM * NH, DH), BF16),
        pltpu.VMEM((DM * NH, DH), BF16),
        pltpu.VMEM((NH * DH, DM), BF16),
        pltpu.VMEM((NB, 16, NH * DH), BF16),
        pltpu.VMEM((NB, 8, NH * DH), F32),
        pltpu.VMEM((NB, NH, DM), F32),
        pltpu.VMEM((NB, NH, SK), F32),
        pltpu.VMEM((NB, NH, 128), F32),
        pltpu.VMEM((NB, NH, 128), F32),
        pltpu.VMEM((NB, NH, DM), F32),
        pltpu.VMEM((16, DM), F32),
        pltpu.SemaphoreType.DMA((G,)),
        pltpu.SemaphoreType.DMA((G,)),
        pltpu.SemaphoreType.DMA((12,)),
        pltpu.SemaphoreType.DMA((4,)),
    ]
    out = pl.pallas_call(
        _kernel,
        out_shape=jax.ShapeDtypeStruct((NB, DM), BF16),
        in_specs=[any_spec] * 11,
        out_specs=pl.BlockSpec(memory_space=pltpu.VMEM),
        scratch_shapes=scratch,
        compiler_params=pltpu.CompilerParams(vmem_limit_bytes=100 * 1024 * 1024),
    )(A_x.reshape(NB, DM), gate_w, k2, v2, A_wq, A_wo, ckv2, bwq2, wuk2, wuv2, bwo2)
    return out.reshape(NB, 1, DM)
```

```python
import jax
import jax.numpy as jnp
from jax import lax
import jax.experimental.pallas as pl
import jax.experimental.pallas.tpu as pltpu

LOOK = 3
BPOS = 1
COMPUTE = True
BCOMP = True
UNR = 16

NB = 2
NH = 32
SK = 8192
DH = 128
DM = 512
NBH = NB * NH
TR = 128
G = 2
NTILE = 64
QT = 16
QROWS = QT * TR
NQ = 4 * NBH

F32 = jnp.float32
BF16 = jnp.bfloat16
NT_DIMS = (((1,), (1,)), ((), ()))


def _tile_order(i):
    return (i % 4) * 16 + i // 4


def _kernel(x_hbm, gate_hbm, k_hbm, v_hbm, wq_hbm, wo_hbm, ckv_hbm, bwq_hbm, wuk_hbm,
            wuv_hbm, bwo_hbm, o_ref,
            x_v, gate_v, kbuf, vbuf, wq_v, wo_v, ckv_v, bwq_v, wuk_v, wuv_v, bwo_v,
            qa_s, oa_s, qabs_s, s_s, m_s, l_s, acc_s, outb_s,
            ksem, vsem, wsem, wosem):
    scale = DH ** -0.5

    def kv_tile(src, dst, sem, item, slot, qd, u):
        i = qd * QT + u
        t = _tile_order(i)
        return pltpu.make_async_copy(
            src.at[pl.ds(pl.multiple_of(item * SK + t * TR, TR), TR)],
            dst.at[slot, pl.ds(pl.multiple_of(i * TR, TR), TR)], sem.at[slot * 4 + qd])

    def issue_kv_quarter(item, qd):
        slot = item % G

        def body(u, c):
            kv_tile(k_hbm, kbuf, ksem, item, slot, qd, u).start(priority=0)
            kv_tile(v_hbm, vbuf, vsem, item, slot, qd, u).start(priority=1)
            return c
        lax.fori_loop(0, QT, body, 0, unroll=UNR)

    def wait_kv_quarter(item, qd):
        slot = item % G
        kb = kbuf.at[slot, pl.ds(qd * QROWS, QROWS)]
        vb = vbuf.at[slot, pl.ds(qd * QROWS, QROWS)]
        pltpu.make_async_copy(kb, kb, ksem.at[slot * 4 + qd]).wait()
        pltpu.make_async_copy(vb, vb, vsem.at[slot * 4 + qd]).wait()

    def rows_tile(src, dst, sem, rows, base, t):
        r0 = pl.multiple_of(base + t * rows, rows)
        return pltpu.make_async_copy(src.at[pl.ds(r0, rows)], dst.at[pl.ds(r0, rows)], sem)

    def issue_extra(item, qd):
        def pairs(src, dst, base0, base1, rows, sem):
            for u in range(4):
                t = _tile_order((item % 4) * QT + qd * 4 + u)
                rows_tile(src, dst, sem, rows, base0, t).start(priority=0)
                rows_tile(src, dst, sem, rows, base1, t).start(priority=1)

        @pl.when(item < 4)
        def _():
            pairs(bwq_hbm, bwq_v, 0, NTILE * TR, TR, wsem.at[1])

        @pl.when(jnp.logical_and(item >= 4, item < 8))
        def _():
            pairs(wuk_hbm, wuk_v, 0, NTILE * TR, TR, wsem.at[2])

        @pl.when(jnp.logical_and(item >= 8, item < 24))
        def _():
            base = pl.multiple_of((item // 4 - 2) * 2048, 2048)
            pairs(ckv_hbm, ckv_v, base, SK + base, 32, wsem.at[3])

        @pl.when(jnp.logical_and(item >= 24, item < 28))
        def _():
            pairs(wuv_hbm, wuv_v, 0, NTILE * TR, TR, wsem.at[4])

        @pl.when(jnp.logical_and(item >= 28, item < 32))
        def _():
            pairs(bwo_hbm, bwo_v, 0, NTILE * 32, 32, wsem.at[5])

    def issue_wq():
        def tile(half, t):
            r0 = pl.multiple_of(half * 256 + (t // 4) * 16, 16)
            c0 = pl.multiple_of((t % 4) * 1024, 1024)
            return pltpu.make_async_copy(
                wq_hbm.at[pl.ds(r0, 16), pl.ds(c0, 1024)],
                wq_v.at[pl.ds(r0, 16), pl.ds(c0, 1024)], wsem.at[0])

        def body(i, c):
            t = _tile_order(i)
            tile(0, t).start(priority=0)
            tile(1, t).start(priority=1)
            return c
        lax.fori_loop(0, NTILE, body, 0, unroll=4)

    def wo_tile(half, i):
        t = _tile_order(i)
        r0 = half * 2048 + t * 32
        return pltpu.make_async_copy(wo_hbm.at[pl.ds(r0, 32)], wo_v.at[pl.ds(r0, 32)],
                                     wosem.at[i // QT])

    def issue_wo_quarter(jq):
        for i in range(QT * jq, QT * jq + QT):
            wo_tile(0, i).start(priority=0)
            wo_tile(1, i).start(priority=1)

    def wait_full(buf, sem):
        pltpu.make_async_copy(buf, buf, sem).wait()

    x_cp = pltpu.make_async_copy(x_hbm, x_v, wsem.at[10])
    g_cp = pltpu.make_async_copy(gate_hbm, gate_v, wsem.at[11])
    x_cp.start()
    g_cp.start()
    issue_wq()
    for n0 in range(LOOK):
        issue_kv_quarter(0, n0)
        issue_extra(jnp.int32(0), n0)

    outb_s[...] = jnp.zeros_like(outb_s)

    x_cp.wait()
    g_cp.wait()
    x2 = x_v[...].astype(F32)
    xf = jnp.concatenate([jnp.broadcast_to(x2[0:1], (8, DM)),
                          jnp.broadcast_to(x2[1:2], (8, DM))], axis=0)
    xb = xf.astype(BF16)
    gate = gate_v[...].astype(F32).reshape(1, DM)
    g = jax.nn.sigmoid(jnp.sum(xf * gate, axis=-1, keepdims=True))

    wait_full(wq_v, wsem.at[0])
    qa = jnp.dot(xb, wq_v[...], preferred_element_type=F32).astype(BF16)
    qa_s[0] = jnp.concatenate([qa[0:8], qa[0:8]], axis=0)
    qa_s[1] = jnp.concatenate([qa[8:16], qa[8:16]], axis=0)

    def deinterleave(w_v, j):
        u = w_v.bitcast(jnp.uint32)[pl.ds(j, DM, stride=NH // 2), :]
        lo = pltpu.bitcast(u << 16, F32).astype(BF16)
        hi = pltpu.bitcast(u & jnp.uint32(0xFFFF0000), F32).astype(BF16)
        return lo, hi

    def b_prologue_group(grp):
        row = lax.broadcasted_iota(jnp.int32, (16, DH), 0) % 8
        tot = None
        for j in range(4 * grp, 4 * grp + 4):
            wq_pair = deinterleave(bwq_v, j)
            wk_pair = deinterleave(wuk_v, j)
            for e in range(2):
                r = (2 * j + e) % 8
                q = jnp.dot(xb, wq_pair[e], preferred_element_type=F32).astype(BF16)
                q = jnp.where(row == r, q, jnp.zeros_like(q))
                qabs = lax.dot_general(q, wk_pair[e], NT_DIMS, preferred_element_type=F32)
                tot = qabs if tot is None else tot + qabs
        qabs_s[0, 8 * grp:8 * grp + 8, :] = tot[0:8]
        qabs_s[1, 8 * grp:8 * grp + 8, :] = tot[8:16]

    CK = 2048

    def b_scores_chunk(b, j):
        q = qabs_s[b].astype(BF16)
        r0 = pl.multiple_of(b * SK + j * CK, CK)
        c = ckv_v[pl.ds(r0, CK), :]
        s = lax.dot_general(q, c, NT_DIMS, preferred_element_type=F32)
        s_s[b, :, pl.ds(pl.multiple_of(j * CK, CK), CK)] = s
        mx = jnp.broadcast_to(jnp.max(s, axis=-1, keepdims=True), (NH, 128))

        @pl.when(j == 0)
        def _():
            m_s[b] = mx

        @pl.when(j > 0)
        def _():
            m_s[b] = jnp.maximum(m_s[b], mx)

    def b_pv_chunk(b, j):
        r0 = pl.multiple_of(b * SK + j * CK, CK)
        c = ckv_v[pl.ds(r0, CK), :]
        s = s_s[b, :, pl.ds(pl.multiple_of(j * CK, CK), CK)]
        m = m_s[b][:, 0:1]
        p = jnp.exp((s - m) * scale)
        ls = jnp.broadcast_to(jnp.sum(p, axis=-1, keepdims=True), (NH, 128))
        pv = jnp.dot(p.astype(BF16), c, preferred_element_type=F32)

        @pl.when(j == 0)
        def _():
            l_s[b] = ls
            acc_s[b] = pv

        @pl.when(j > 0)
        def _():
            l_s[b] = l_s[b] + ls
            acc_s[b] = acc_s[b] + pv

    def b_normalize():
        for b in range(NB):
            acc_s[b] = acc_s[b] / l_s[b][:, 0:1]

    def b_epilogue_group(grp):
        row = lax.broadcasted_iota(jnp.int32, (16, DH), 0) % 8
        lhs = jnp.concatenate([acc_s[0, 8 * grp:8 * grp + 8, :], acc_s[1, 8 * grp:8 * grp + 8, :]],
                              axis=0).astype(BF16)
        tot = None
        for j in range(4 * grp, 4 * grp + 4):
            wv_pair = deinterleave(wuv_v, j)
            for e in range(2):
                h = 2 * j + e
                ctx = jnp.dot(lhs, wv_pair[e], preferred_element_type=F32).astype(BF16)
                ctx = jnp.where(row == h % 8, ctx, jnp.zeros_like(ctx))
                part = jnp.dot(ctx, bwo_v[h * DH:(h + 1) * DH, :], preferred_element_type=F32)
                tot = part if tot is None else tot + part
        outb_s[...] += tot

    def a_step(s):
        b = s // NH
        h = s % NH
        slot = s % G
        c0 = pl.multiple_of(h * DH, DH)
        q = qa_s[b, :, pl.ds(c0, DH)]
        sc = lax.dot_general(q, kbuf[slot], NT_DIMS, preferred_element_type=F32)
        m = jnp.max(sc, axis=-1, keepdims=True)
        p = jnp.exp((sc - m) * scale)
        l = jnp.sum(p, axis=-1, keepdims=True)
        o = jnp.dot(p.astype(BF16), vbuf[slot], preferred_element_type=F32)
        o = o / l
        oa_s[b, :, pl.ds(c0, DH)] = o[0:8, :]

    S_BPRO = 8
    S_BSC = 24
    S_BPV = S_BSC + 8
    S_BEPI = S_BPV + 8

    def b_work(s):
        @pl.when(s == S_BPRO)
        def _():
            wait_full(bwq_v, wsem.at[1])
            wait_full(wuk_v, wsem.at[2])

        if BCOMP:
            for grp in range(4):
                pl.when(s == S_BPRO + grp)(lambda grp=grp: b_prologue_group(grp))

        @pl.when(s == S_BSC)
        def _():
            wait_full(ckv_v, wsem.at[3])

        if BCOMP:
            @pl.when(jnp.logical_and(s >= S_BSC, s < S_BSC + 8))
            def _():
                i = s - S_BSC
                b_scores_chunk(i // 4, i % 4)

            @pl.when(jnp.logical_and(s >= S_BPV, s < S_BPV + 8))
            def _():
                i = s - S_BPV
                b_pv_chunk(i // 4, i % 4)

        @pl.when(s == S_BEPI)
        def _():
            wait_full(wuv_v, wsem.at[4])
            wait_full(bwo_v, wsem.at[5])
            if BCOMP:
                b_normalize()

        if BCOMP:
            for grp in range(4):
                pl.when(s == S_BEPI + grp)(lambda grp=grp: b_epilogue_group(grp))

    def step(s, carry):
        for qd in range(4):
            wait_kv_quarter(s, qd)
            di, nq = (qd + LOOK) // 4, (qd + LOOK) % 4
            item = s + di
            if di == 0:
                issue_kv_quarter(item, nq)
                issue_extra(item, nq)
            else:
                @pl.when(item < NBH)
                def _():
                    issue_kv_quarter(item, nq)
                    issue_extra(item, nq)

                @pl.when(item == NBH)
                def _():
                    issue_wo_quarter(nq)
            if qd == BPOS:
                b_work(s)

        if COMPUTE:
            a_step(s)
        return carry

    lax.fori_loop(0, NBH, step, 0)

    for jq in range(LOOK, 4):
        issue_wo_quarter(jq)
    if not COMPUTE:
        oa_s[...] = jnp.zeros_like(oa_s)
    oa = jnp.concatenate([oa_s[0], oa_s[1]], axis=0).astype(BF16)
    acc = jnp.zeros((16, DM), F32)
    for jq in range(4):
        for i in range(QT * jq, QT * jq + QT):
            wo_tile(0, i).wait()
            wo_tile(1, i).wait()
        for half in range(2):
            for st in range(4):
                hd = half * 16 + st * 4 + jq
                acc = acc + jnp.dot(oa[:, hd * DH:(hd + 1) * DH],
                                    wo_v[hd * DH:(hd + 1) * DH, :],
                                    preferred_element_type=F32)
    a_out = acc.astype(BF16).astype(F32)
    ob = outb_s[...]
    b0 = jnp.sum(ob[0:8], axis=0, keepdims=True).astype(BF16).astype(F32)
    b1 = jnp.sum(ob[8:16], axis=0, keepdims=True).astype(BF16).astype(F32)
    g0 = g[0:1, :]
    g1 = g[8:9, :]
    r0 = g0 * a_out[0:1, :] + (1.0 - g0) * b0
    r1 = g1 * a_out[8:9, :] + (1.0 - g1) * b1
    o_ref[...] = jnp.concatenate([r0, r1], axis=0).astype(o_ref.dtype)


@jax.jit
def pallas_gated_mix__mha_block_cached__compressed_kv_cla__decode_kernel(
    A_x, A_k_cache, A_v_cache, A_wq, A_wo, B_x, B_c_kv, B_w_q, B_w_uk, B_w_uv, B_w_o, gate_w,
):
    del B_x
    k2 = A_k_cache.reshape(NBH * SK, DH)
    v2 = A_v_cache.reshape(NBH * SK, DH)
    ckv2 = B_c_kv.reshape(NB * SK, DM)
    bwq2 = B_w_q.reshape(DM * NH, DH)
    wuk2 = B_w_uk.reshape(DM * NH, DH)
    wuv2 = B_w_uv.reshape(DM * NH, DH)
    bwo2 = B_w_o.reshape(NH * DH, DM)

    any_spec = pl.BlockSpec(memory_space=pl.ANY)
    scratch = [
        pltpu.VMEM((NB, DM), BF16),
        pltpu.VMEM((DM,), BF16),
        pltpu.VMEM((G, SK, DH), BF16),
        pltpu.VMEM((G, SK, DH), BF16),
        pltpu.VMEM((DM, NH * DH), BF16),
        pltpu.VMEM((NH * DH, DM), BF16),
        pltpu.VMEM((NB * SK, DM), BF16),
        pltpu.VMEM((DM * NH, DH), BF16),
        pltpu.VMEM((DM * NH, DH), BF16),
        pltpu.VMEM((DM * NH, DH), BF16),
        pltpu.VMEM((NH * DH, DM), BF16),
        pltpu.VMEM((NB, 16, NH * DH), BF16),
        pltpu.VMEM((NB, 8, NH * DH), F32),
        pltpu.VMEM((NB, NH, DM), F32),
        pltpu.VMEM((NB, NH, SK), F32),
        pltpu.VMEM((NB, NH, 128), F32),
        pltpu.VMEM((NB, NH, 128), F32),
        pltpu.VMEM((NB, NH, DM), F32),
        pltpu.VMEM((16, DM), F32),
        pltpu.SemaphoreType.DMA((G * 4,)),
        pltpu.SemaphoreType.DMA((G * 4,)),
        pltpu.SemaphoreType.DMA((12,)),
        pltpu.SemaphoreType.DMA((4,)),
    ]
    out = pl.pallas_call(
        _kernel,
        out_shape=jax.ShapeDtypeStruct((NB, DM), BF16),
        in_specs=[any_spec] * 11,
        out_specs=pl.BlockSpec(memory_space=pltpu.VMEM),
        scratch_shapes=scratch,
        compiler_params=pltpu.CompilerParams(vmem_limit_bytes=100 * 1024 * 1024),
    )(A_x.reshape(NB, DM), gate_w, k2, v2, A_wq, A_wo, ckv2, bwq2, wuk2, wuv2, bwo2)
    return out.reshape(NB, 1, DM)
```

```python
import jax
import jax.numpy as jnp
from jax import lax
import jax.experimental.pallas as pl
import jax.experimental.pallas.tpu as pltpu

NB = 2
NH = 32
SK = 8192
DH = 128
DM = 512
NBH = NB * NH

TR = 128
WR = 32
NT = 64
QT = 16
NGRP = NT // QT
GROWS = QT * TR
XP = QT // 4
NSLOT = 2
CK = 2048

WO_GROUPS = ((0, 4, 8, 12), (1, 5, 9, 13), (2, 6, 10, 14), (3, 7, 11), (15,))
WO_IN_LOOP = 3

S_BPRO = 8
S_BSC = 24
S_BPV = S_BSC + 8
S_BEPI = S_BPV + 8

F32 = jnp.float32
BF16 = jnp.bfloat16
NT_DIMS = (((1,), (1,)), ((), ()))


def _stream_order(i):
    return (i % 4) * 16 + i // 4


def _kernel(x_hbm, gate_hbm, k_hbm, v_hbm, wq_hbm, wo_hbm, ckv_hbm, bwq_hbm, wuk_hbm,
            wuv_hbm, bwo_hbm, o_ref,
            x_v, gate_v, kbuf, vbuf, wq_v, wo_v, ckv_v, bwq_v, wuk_v, wuv_v, bwo_v,
            qa_s, oa_s, qabs_s, s_s, m_s, l_s, acc_s, outb_s,
            ksem, vsem, wsem, wosem):
    scale = DH ** -0.5

    def kv_tile(src, dst, sem, item, slot, grp, u):
        i = grp * QT + u
        return pltpu.make_async_copy(
            src.at[pl.ds(pl.multiple_of(item * SK + _stream_order(i) * TR, TR), TR)],
            dst.at[slot, pl.ds(i * TR, TR)],
            sem.at[slot * NGRP + grp])

    def issue_kv_group(item, grp):
        slot = item & (NSLOT - 1)
        for u in range(QT):
            kv_tile(k_hbm, kbuf, ksem, item, slot, grp, u).start(priority=0)
            kv_tile(v_hbm, vbuf, vsem, item, slot, grp, u).start(priority=1)

    def wait_kv_group(item, grp):
        slot = item & (NSLOT - 1)
        kb = kbuf.at[slot, pl.ds(grp * GROWS, GROWS)]
        vb = vbuf.at[slot, pl.ds(grp * GROWS, GROWS)]
        pltpu.make_async_copy(kb, kb, ksem.at[slot * NGRP + grp]).wait()
        pltpu.make_async_copy(vb, vb, vsem.at[slot * NGRP + grp]).wait()

    def rows_tile(src, dst, sem, rows, base, t):
        r0 = pl.multiple_of(base + t * rows, rows)
        return pltpu.make_async_copy(src.at[pl.ds(r0, rows)], dst.at[pl.ds(r0, rows)], sem)

    def issue_b_operands(item, grp):
        def pairs(src, dst, base0, base1, rows, sem):
            dyn = (item & 3) * 4
            for u in range(XP):
                c = grp * XP + u
                t = dyn + ((c % 4) * 16 + c // 4)
                rows_tile(src, dst, sem, rows, base0, t).start(priority=0)
                rows_tile(src, dst, sem, rows, base1, t).start(priority=1)

        @pl.when(item < 4)
        def _():
            pairs(bwq_hbm, bwq_v, 0, NT * TR, TR, wsem.at[1])

        @pl.when(jnp.logical_and(item >= 4, item < 8))
        def _():
            pairs(wuk_hbm, wuk_v, 0, NT * TR, TR, wsem.at[2])

        @pl.when(jnp.logical_and(item >= 8, item < 24))
        def _():
            base = pl.multiple_of(((item >> 2) - 2) * CK, CK)
            pairs(ckv_hbm, ckv_v, base, SK + base, WR, wsem.at[3])

        @pl.when(jnp.logical_and(item >= 24, item < 28))
        def _():
            pairs(wuv_hbm, wuv_v, 0, NT * TR, TR, wsem.at[4])

        @pl.when(jnp.logical_and(item >= 28, item < 32))
        def _():
            pairs(bwo_hbm, bwo_v, 0, NT * WR, WR, wsem.at[5])

    def issue_wq():
        def tile(half, t):
            r0 = pl.multiple_of(half * 256 + (t >> 1) * 8, 8)
            c0 = pl.multiple_of((t & 1) * 2048, 2048)
            return pltpu.make_async_copy(
                wq_hbm.at[pl.ds(r0, 8), pl.ds(c0, 2048)],
                wq_v.at[pl.ds(r0, 8), pl.ds(c0, 2048)], wsem.at[0])

        def body(i, c):
            t = (i & 3) * 16 + (i >> 2)
            tile(0, t).start(priority=0)
            tile(1, t).start(priority=1)
            return c
        lax.fori_loop(0, NT, body, 0, unroll=4)

    def wo_tiles(gi):
        out = []
        for p in range(DH // WR):
            for hd in WO_GROUPS[gi]:
                for half in range(2):
                    r0 = (half * 16 + hd) * DH + p * WR
                    out.append((half, pltpu.make_async_copy(
                        wo_hbm.at[pl.ds(r0, WR)], wo_v.at[pl.ds(r0, WR)], wosem.at[gi])))
        return out

    def issue_wo_group(gi):
        for half, cp in wo_tiles(gi):
            cp.start(priority=half)

    def wait_full(buf, sem):
        pltpu.make_async_copy(buf, buf, sem).wait()

    x_cp = pltpu.make_async_copy(x_hbm, x_v, wsem.at[6])
    g_cp = pltpu.make_async_copy(gate_hbm, gate_v, wsem.at[7])
    x_cp.start()
    g_cp.start()
    issue_wq()
    for grp in range(NGRP):
        issue_kv_group(0, grp)
        issue_b_operands(jnp.int32(0), grp)

    outb_s[...] = jnp.zeros_like(outb_s)

    x_cp.wait()
    g_cp.wait()
    x2 = x_v[...].astype(F32)
    xf = jnp.concatenate([jnp.broadcast_to(x2[0:1], (8, DM)),
                          jnp.broadcast_to(x2[1:2], (8, DM))], axis=0)
    xb = xf.astype(BF16)
    gate = gate_v[...].astype(F32).reshape(1, DM)
    g = jax.nn.sigmoid(jnp.sum(xf * gate, axis=-1, keepdims=True))

    wait_full(wq_v, wsem.at[0])
    qa = jnp.dot(xb, wq_v[...], preferred_element_type=F32).astype(BF16)
    qa_s[0] = jnp.concatenate([qa[0:8], qa[0:8]], axis=0)
    qa_s[1] = jnp.concatenate([qa[8:16], qa[8:16]], axis=0)

    def deinterleave(w_v, j):
        u = w_v.bitcast(jnp.uint32)[pl.ds(j, DM, stride=NH // 2), :]
        lo = pltpu.bitcast(u << 16, F32).astype(BF16)
        hi = pltpu.bitcast(u & jnp.uint32(0xFFFF0000), F32).astype(BF16)
        return lo, hi

    def b_queries(grp):
        row = lax.broadcasted_iota(jnp.int32, (16, DH), 0) % 8
        tot = None
        for j in range(4 * grp, 4 * grp + 4):
            wq_pair = deinterleave(bwq_v, j)
            wk_pair = deinterleave(wuk_v, j)
            for e in range(2):
                q = jnp.dot(xb, wq_pair[e], preferred_element_type=F32).astype(BF16)
                q = jnp.where(row == (2 * j + e) % 8, q, jnp.zeros_like(q))
                qabs = lax.dot_general(q, wk_pair[e], NT_DIMS, preferred_element_type=F32)
                tot = qabs if tot is None else tot + qabs
        qabs_s[0, 8 * grp:8 * grp + 8, :] = tot[0:8]
        qabs_s[1, 8 * grp:8 * grp + 8, :] = tot[8:16]

    def b_scores(b, j):
        q = qabs_s[b].astype(BF16)
        c = ckv_v[pl.ds(pl.multiple_of(b * SK + j * CK, CK), CK), :]
        s = lax.dot_general(q, c, NT_DIMS, preferred_element_type=F32)
        s_s[b, :, pl.ds(pl.multiple_of(j * CK, CK), CK)] = s
        mx = jnp.broadcast_to(jnp.max(s, axis=-1, keepdims=True), (NH, 128))

        @pl.when(j == 0)
        def _():
            m_s[b] = mx

        @pl.when(j > 0)
        def _():
            m_s[b] = jnp.maximum(m_s[b], mx)

    def b_context(b, j):
        c = ckv_v[pl.ds(pl.multiple_of(b * SK + j * CK, CK), CK), :]
        s = s_s[b, :, pl.ds(pl.multiple_of(j * CK, CK), CK)]
        p = jnp.exp((s - m_s[b][:, 0:1]) * scale)
        ls = jnp.broadcast_to(jnp.sum(p, axis=-1, keepdims=True), (NH, 128))
        pv = jnp.dot(p.astype(BF16), c, preferred_element_type=F32)

        @pl.when(j == 0)
        def _():
            l_s[b] = ls
            acc_s[b] = pv

        @pl.when(j > 0)
        def _():
            l_s[b] = l_s[b] + ls
            acc_s[b] = acc_s[b] + pv

    def b_normalize():
        for b in range(NB):
            acc_s[b] = acc_s[b] / l_s[b][:, 0:1]

    def b_output(grp):
        row = lax.broadcasted_iota(jnp.int32, (16, DH), 0) % 8
        lhs = jnp.concatenate([acc_s[0, 8 * grp:8 * grp + 8, :],
                               acc_s[1, 8 * grp:8 * grp + 8, :]], axis=0).astype(BF16)
        tot = None
        for j in range(4 * grp, 4 * grp + 4):
            wv_pair = deinterleave(wuv_v, j)
            for e in range(2):
                h = 2 * j + e
                ctx = jnp.dot(lhs, wv_pair[e], preferred_element_type=F32).astype(BF16)
                ctx = jnp.where(row == h % 8, ctx, jnp.zeros_like(ctx))
                part = jnp.dot(ctx, bwo_v[h * DH:(h + 1) * DH, :], preferred_element_type=F32)
                tot = part if tot is None else tot + part
        outb_s[...] += tot

    def b_work(s):
        @pl.when(s == S_BPRO)
        def _():
            wait_full(bwq_v, wsem.at[1])
            wait_full(wuk_v, wsem.at[2])

        for grp in range(4):
            pl.when(s == S_BPRO + grp)(lambda grp=grp: b_queries(grp))

        @pl.when(s == S_BSC)
        def _():
            wait_full(ckv_v, wsem.at[3])

        @pl.when(jnp.logical_and(s >= S_BSC, s < S_BPV))
        def _():
            i = s - S_BSC
            b_scores(i >> 2, i & 3)

        @pl.when(jnp.logical_and(s >= S_BPV, s < S_BEPI))
        def _():
            i = s - S_BPV
            b_context(i >> 2, i & 3)

        @pl.when(s == S_BEPI)
        def _():
            wait_full(wuv_v, wsem.at[4])
            wait_full(bwo_v, wsem.at[5])
            b_normalize()

        for grp in range(4):
            pl.when(s == S_BEPI + grp)(lambda grp=grp: b_output(grp))

    def a_item(s):
        b = s >> 5
        h = s & (NH - 1)
        slot = s & (NSLOT - 1)
        c0 = pl.multiple_of(h * DH, DH)
        q = qa_s[b, :, pl.ds(c0, DH)]
        sc = lax.dot_general(q, kbuf[slot], NT_DIMS, preferred_element_type=F32)
        m = jnp.max(sc, axis=-1, keepdims=True)
        p = jnp.exp((sc - m) * scale)
        l = jnp.sum(p, axis=-1, keepdims=True)
        o = jnp.dot(p.astype(BF16), vbuf[slot], preferred_element_type=F32)
        oa_s[b, :, pl.ds(c0, DH)] = (o / l)[0:8, :]

    def step(s, carry):
        nxt = s + 1
        for grp in range(NGRP):
            wait_kv_group(s, grp)

            @pl.when(nxt < NBH)
            def _():
                issue_kv_group(nxt, grp)
                issue_b_operands(nxt, grp)

            if grp < WO_IN_LOOP:
                @pl.when(nxt == NBH)
                def _():
                    issue_wo_group(grp)

            if grp == 0:
                b_work(s)

        a_item(s)
        return carry

    lax.fori_loop(0, NBH, step, 0)

    for gi in range(WO_IN_LOOP, len(WO_GROUPS)):
        issue_wo_group(gi)

    ob = outb_s[...]
    b0 = jnp.sum(ob[0:8], axis=0, keepdims=True).astype(BF16).astype(F32)
    b1 = jnp.sum(ob[8:16], axis=0, keepdims=True).astype(BF16).astype(F32)
    g0 = g[0:1, :]
    g1 = g[8:9, :]
    t0 = (1.0 - g0) * b0
    t1 = (1.0 - g1) * b1

    oa = jnp.concatenate([oa_s[0], oa_s[1]], axis=0).astype(BF16)
    acc = jnp.zeros((16, DM), F32)
    for gi in range(len(WO_GROUPS)):
        for _, cp in wo_tiles(gi):
            cp.wait()
        for hd0 in WO_GROUPS[gi]:
            for half in range(2):
                hd = half * 16 + hd0
                acc = acc + jnp.dot(oa[:, hd * DH:(hd + 1) * DH],
                                    wo_v[hd * DH:(hd + 1) * DH, :],
                                    preferred_element_type=F32)
    a_out = acc.astype(BF16).astype(F32)
    r0 = g0 * a_out[0:1, :] + t0
    r1 = g1 * a_out[8:9, :] + t1
    o_ref[...] = jnp.concatenate([r0, r1], axis=0).astype(o_ref.dtype)


@jax.jit
def pallas_gated_mix__mha_block_cached__compressed_kv_cla__decode_kernel(
    A_x: jax.Array,
    A_k_cache: jax.Array,
    A_v_cache: jax.Array,
    A_wq: jax.Array,
    A_wo: jax.Array,
    B_x: jax.Array,
    B_c_kv: jax.Array,
    B_w_q: jax.Array,
    B_w_uk: jax.Array,
    B_w_uv: jax.Array,
    B_w_o: jax.Array,
    gate_w: jax.Array,
):
    del B_x
    k2 = A_k_cache.reshape(NBH * SK, DH)
    v2 = A_v_cache.reshape(NBH * SK, DH)
    ckv2 = B_c_kv.reshape(NB * SK, DM)
    bwq2 = B_w_q.reshape(DM * NH, DH)
    wuk2 = B_w_uk.reshape(DM * NH, DH)
    wuv2 = B_w_uv.reshape(DM * NH, DH)
    bwo2 = B_w_o.reshape(NH * DH, DM)

    any_spec = pl.BlockSpec(memory_space=pl.ANY)
    scratch = [
        pltpu.VMEM((NB, DM), BF16),
        pltpu.VMEM((DM,), BF16),
        pltpu.VMEM((NSLOT, SK, DH), BF16),
        pltpu.VMEM((NSLOT, SK, DH), BF16),
        pltpu.VMEM((DM, NH * DH), BF16),
        pltpu.VMEM((NH * DH, DM), BF16),
        pltpu.VMEM((NB * SK, DM), BF16),
        pltpu.VMEM((DM * NH, DH), BF16),
        pltpu.VMEM((DM * NH, DH), BF16),
        pltpu.VMEM((DM * NH, DH), BF16),
        pltpu.VMEM((NH * DH, DM), BF16),
        pltpu.VMEM((NB, 16, NH * DH), BF16),
        pltpu.VMEM((NB, 8, NH * DH), F32),
        pltpu.VMEM((NB, NH, DM), F32),
        pltpu.VMEM((NB, NH, SK), F32),
        pltpu.VMEM((NB, NH, 128), F32),
        pltpu.VMEM((NB, NH, 128), F32),
        pltpu.VMEM((NB, NH, DM), F32),
        pltpu.VMEM((16, DM), F32),
        pltpu.SemaphoreType.DMA((NSLOT * NGRP,)),
        pltpu.SemaphoreType.DMA((NSLOT * NGRP,)),
        pltpu.SemaphoreType.DMA((8,)),
        pltpu.SemaphoreType.DMA((len(WO_GROUPS),)),
    ]
    out = pl.pallas_call(
        _kernel,
        out_shape=jax.ShapeDtypeStruct((NB, DM), BF16),
        in_specs=[any_spec] * 11,
        out_specs=pl.BlockSpec(memory_space=pltpu.VMEM),
        scratch_shapes=scratch,
        compiler_params=pltpu.CompilerParams(vmem_limit_bytes=100 * 1024 * 1024),
    )(A_x.reshape(NB, DM), gate_w, k2, v2, A_wq, A_wo, ckv2, bwq2, wuk2, wuv2, bwo2)
    return out.reshape(NB, 1, DM)
```

```python
import jax
import jax.numpy as jnp
from jax import lax
import jax.experimental.pallas as pl
import jax.experimental.pallas.tpu as pltpu

NB = 2
NH = 32
SK = 8192
DH = 128
DM = 512
NBH = NB * NH

TR = 128
WR = 32
NT = 64
QT = 16
NGRP = NT // QT
GROWS = QT * TR
NXB = 8
NSLOT = 2
CK = 2048

WO_GROUPS = ((0, 4, 8, 12), (1, 5, 9, 13), (2, 6, 10, 14), (3, 7, 11), (15,))
WO_IN_LOOP = 3

S_BPRO = 10
S_BSC = 16
S_BPV = S_BSC + 8
S_BEPI = S_BPV + 9

F32 = jnp.float32
BF16 = jnp.bfloat16
NT_DIMS = (((1,), (1,)), ((), ()))


def _stream_order(i):
    return (i % 4) * 16 + i // 4


def _kernel(x_hbm, gate_hbm, k_hbm, v_hbm, wq_hbm, wo_hbm, ckv_hbm, bwq_hbm, wuk_hbm,
            wuv_hbm, bwo_hbm, o_ref,
            x_v, gate_v, kbuf, vbuf, wq_v, wo_v, ckv_v, bwq_v, wuk_v, wuv_v, bwo_v,
            ua_s, ub_s, qa_s, oa_s, qabs_s, s_s, m_s, l_s, acc_s, outb_s,
            ksem, vsem, wsem, wosem):
    scale = DH ** -0.5

    def kv_tile(src, dst, sem, item, slot, grp, u):
        i = grp * QT + u
        return pltpu.make_async_copy(
            src.at[pl.ds(pl.multiple_of(item * SK + _stream_order(i) * TR, TR), TR)],
            dst.at[slot, pl.ds(i * TR, TR)],
            sem.at[slot * NGRP + grp])

    def issue_kv_group(item, grp):
        slot = item & (NSLOT - 1)
        for u in range(QT):
            kv_tile(k_hbm, kbuf, ksem, item, slot, grp, u).start(priority=0)
            kv_tile(v_hbm, vbuf, vsem, item, slot, grp, u).start(priority=1)

    def wait_kv_group(item, grp):
        slot = item & (NSLOT - 1)
        kb = kbuf.at[slot, pl.ds(grp * GROWS, GROWS)]
        vb = vbuf.at[slot, pl.ds(grp * GROWS, GROWS)]
        pltpu.make_async_copy(kb, kb, ksem.at[slot * NGRP + grp]).wait()
        pltpu.make_async_copy(vb, vb, vsem.at[slot * NGRP + grp]).wait()

    def rows_tile(src, dst, sem, rows, base, t):
        r0 = pl.multiple_of(base + t * rows, rows)
        return pltpu.make_async_copy(src.at[pl.ds(r0, rows)], dst.at[pl.ds(r0, rows)], sem)

    def issue_b_group(sx, grp):
        def pairs(src, dst, base0, base1, rows, sem):
            for u in range(QT):
                t = _stream_order(grp * QT + u)
                rows_tile(src, dst, sem, rows, base0, t).start(priority=0)
                rows_tile(src, dst, sem, rows, base1, t).start(priority=1)

        @pl.when(sx == 0)
        def _():
            pairs(bwq_hbm, bwq_v, 0, NT * TR, TR, wsem.at[1])

        @pl.when(sx == 1)
        def _():
            pairs(wuk_hbm, wuk_v, 0, NT * TR, TR, wsem.at[2])

        @pl.when(jnp.logical_and(sx >= 2, sx < 6))
        def _():
            base = pl.multiple_of((sx - 2) * CK, CK)
            pairs(ckv_hbm, ckv_v, base, SK + base, WR, wsem.at[3])

        @pl.when(sx == 6)
        def _():
            pairs(wuv_hbm, wuv_v, 0, NT * TR, TR, wsem.at[4])

        @pl.when(sx == 7)
        def _():
            pairs(bwo_hbm, bwo_v, 0, NT * WR, WR, wsem.at[5])

    def issue_wq():
        def tile(half, t):
            r0 = pl.multiple_of(half * 256 + (t >> 1) * 8, 8)
            c0 = pl.multiple_of((t & 1) * 2048, 2048)
            return pltpu.make_async_copy(
                wq_hbm.at[pl.ds(r0, 8), pl.ds(c0, 2048)],
                wq_v.at[pl.ds(r0, 8), pl.ds(c0, 2048)], wsem.at[0])

        def body(i, c):
            t = (i & 3) * 16 + (i >> 2)
            tile(0, t).start(priority=0)
            tile(1, t).start(priority=1)
            return c
        lax.fori_loop(0, NT, body, 0, unroll=4)

    def wo_tiles(gi):
        out = []
        for p in range(DH // WR):
            for hd in WO_GROUPS[gi]:
                for half in range(2):
                    r0 = (half * 16 + hd) * DH + p * WR
                    out.append((half, pltpu.make_async_copy(
                        wo_hbm.at[pl.ds(r0, WR)], wo_v.at[pl.ds(r0, WR)], wosem.at[gi])))
        return out

    def issue_wo_group(gi):
        for half, cp in wo_tiles(gi):
            cp.start(priority=half)

    def wait_full(buf, sem):
        pltpu.make_async_copy(buf, buf, sem).wait()

    x_cp = pltpu.make_async_copy(x_hbm, x_v, wsem.at[6])
    g_cp = pltpu.make_async_copy(gate_hbm, gate_v, wsem.at[7])
    x_cp.start()
    g_cp.start()
    issue_wq()
    for grp in range(NGRP):
        issue_kv_group(0, grp)

    outb_s[...] = jnp.zeros_like(outb_s)

    x_cp.wait()
    g_cp.wait()
    x2 = x_v[...].astype(F32)
    xf = jnp.concatenate([jnp.broadcast_to(x2[0:1], (8, DM)),
                          jnp.broadcast_to(x2[1:2], (8, DM))], axis=0)
    xb = xf.astype(BF16)
    gate = gate_v[...].astype(F32).reshape(1, DM)
    g = jax.nn.sigmoid(jnp.sum(xf * gate, axis=-1, keepdims=True))

    wait_full(wq_v, wsem.at[0])
    qa = jnp.dot(xb, wq_v[...], preferred_element_type=F32).astype(BF16)
    qa_s[0] = jnp.concatenate([qa[0:8], qa[0:8]], axis=0)
    qa_s[1] = jnp.concatenate([qa[8:16], qa[8:16]], axis=0)

    def to_words(w_v, u_s):
        def body(i, c):
            x = w_v[pl.ds(pl.multiple_of(i * 1024, 1024), 1024), :]
            u_s[pl.ds(pl.multiple_of(i * 512, 512), 512), :] = pltpu.bitcast(x, jnp.uint32)
            return c
        lax.fori_loop(0, DM * NH // 1024, body, 0)

    def deinterleave(u_s, j):
        u = u_s[pl.ds(j, DM, stride=NH // 2), :]
        lo = pltpu.bitcast(u << 16, F32).astype(BF16)
        hi = pltpu.bitcast(u & jnp.uint32(0xFFFF0000), F32).astype(BF16)
        return lo, hi

    def b_queries(grp):
        row = lax.broadcasted_iota(jnp.int32, (16, DH), 0) % 8
        tot = None
        for j in range(4 * grp, 4 * grp + 4):
            wq_pair = deinterleave(ua_s, j)
            wk_pair = deinterleave(ub_s, j)
            for e in range(2):
                q = jnp.dot(xb, wq_pair[e], preferred_element_type=F32).astype(BF16)
                q = jnp.where(row == (2 * j + e) % 8, q, jnp.zeros_like(q))
                qabs = lax.dot_general(q, wk_pair[e], NT_DIMS, preferred_element_type=F32)
                tot = qabs if tot is None else tot + qabs
        qabs_s[0, 8 * grp:8 * grp + 8, :] = tot[0:8]
        qabs_s[1, 8 * grp:8 * grp + 8, :] = tot[8:16]

    def b_scores(b, j):
        q = qabs_s[b].astype(BF16)
        c = ckv_v[pl.ds(pl.multiple_of(b * SK + j * CK, CK), CK), :]
        s = lax.dot_general(q, c, NT_DIMS, preferred_element_type=F32)
        s_s[b, :, pl.ds(pl.multiple_of(j * CK, CK), CK)] = s
        mx = jnp.broadcast_to(jnp.max(s, axis=-1, keepdims=True), (NH, 128))

        @pl.when(j == 0)
        def _():
            m_s[b] = mx

        @pl.when(j > 0)
        def _():
            m_s[b] = jnp.maximum(m_s[b], mx)

    def b_context(b, j):
        c = ckv_v[pl.ds(pl.multiple_of(b * SK + j * CK, CK), CK), :]
        s = s_s[b, :, pl.ds(pl.multiple_of(j * CK, CK), CK)]
        p = jnp.exp((s - m_s[b][:, 0:1]) * scale)
        ls = jnp.broadcast_to(jnp.sum(p, axis=-1, keepdims=True), (NH, 128))
        pv = jnp.dot(p.astype(BF16), c, preferred_element_type=F32)

        @pl.when(j == 0)
        def _():
            l_s[b] = ls
            acc_s[b] = pv

        @pl.when(j > 0)
        def _():
            l_s[b] = l_s[b] + ls
            acc_s[b] = acc_s[b] + pv

    def b_normalize():
        for b in range(NB):
            acc_s[b] = acc_s[b] / l_s[b][:, 0:1]

    def b_output(grp):
        row = lax.broadcasted_iota(jnp.int32, (16, DH), 0) % 8
        lhs = jnp.concatenate([acc_s[0, 8 * grp:8 * grp + 8, :],
                               acc_s[1, 8 * grp:8 * grp + 8, :]], axis=0).astype(BF16)
        tot = None
        for j in range(4 * grp, 4 * grp + 4):
            wv_pair = deinterleave(ua_s, j)
            for e in range(2):
                h = 2 * j + e
                ctx = jnp.dot(lhs, wv_pair[e], preferred_element_type=F32).astype(BF16)
                ctx = jnp.where(row == h % 8, ctx, jnp.zeros_like(ctx))
                part = jnp.dot(ctx, bwo_v[h * DH:(h + 1) * DH, :], preferred_element_type=F32)
                tot = part if tot is None else tot + part
        outb_s[...] += tot

    def b_work(s):
        @pl.when(s == S_BPRO - 2)
        def _():
            wait_full(bwq_v, wsem.at[1])
            to_words(bwq_v, ua_s)

        @pl.when(s == S_BPRO - 1)
        def _():
            wait_full(wuk_v, wsem.at[2])
            to_words(wuk_v, ub_s)

        for grp in range(4):
            pl.when(s == S_BPRO + grp)(lambda grp=grp: b_queries(grp))

        @pl.when(s == S_BSC)
        def _():
            wait_full(ckv_v, wsem.at[3])

        @pl.when(jnp.logical_and(s >= S_BSC, s < S_BPV))
        def _():
            i = s - S_BSC
            b_scores(i >> 2, i & 3)

        @pl.when(jnp.logical_and(s >= S_BPV, s < S_BPV + 8))
        def _():
            i = s - S_BPV
            b_context(i >> 2, i & 3)

        @pl.when(s == S_BEPI - 1)
        def _():
            wait_full(wuv_v, wsem.at[4])
            to_words(wuv_v, ua_s)

        @pl.when(s == S_BEPI)
        def _():
            wait_full(bwo_v, wsem.at[5])
            b_normalize()

        for grp in range(4):
            pl.when(s == S_BEPI + grp)(lambda grp=grp: b_output(grp))

    def a_item(s):
        b = s >> 5
        h = s & (NH - 1)
        slot = s & (NSLOT - 1)
        c0 = pl.multiple_of(h * DH, DH)
        q = qa_s[b, :, pl.ds(c0, DH)]
        sc = lax.dot_general(q, kbuf[slot], NT_DIMS, preferred_element_type=F32)
        m = jnp.max(sc, axis=-1, keepdims=True)
        p = jnp.exp((sc - m) * scale)
        l = jnp.sum(p, axis=-1, keepdims=True)
        o = jnp.dot(p.astype(BF16), vbuf[slot], preferred_element_type=F32)
        oa_s[b, :, pl.ds(c0, DH)] = (o / l)[0:8, :]

    def step(s, carry):
        nxt = s + 1
        has_b = s < NXB
        for grp in range(NGRP):
            wait_kv_group(s, grp)

            @pl.when(has_b)
            def _():
                issue_b_group(s, grp)

            @pl.when(jnp.logical_and(jnp.logical_not(has_b), nxt < NBH))
            def _():
                issue_kv_group(nxt, grp)

            if grp < WO_IN_LOOP:
                @pl.when(nxt == NBH)
                def _():
                    issue_wo_group(grp)

            if grp == 0:
                b_work(s)

        a_item(s)

        @pl.when(has_b)
        def _():
            for grp in range(NGRP):
                issue_kv_group(nxt, grp)
        return carry

    lax.fori_loop(0, NBH, step, 0)

    for gi in range(WO_IN_LOOP, len(WO_GROUPS)):
        issue_wo_group(gi)

    ob = outb_s[...]
    b0 = jnp.sum(ob[0:8], axis=0, keepdims=True).astype(BF16).astype(F32)
    b1 = jnp.sum(ob[8:16], axis=0, keepdims=True).astype(BF16).astype(F32)
    g0 = g[0:1, :]
    g1 = g[8:9, :]
    t0 = (1.0 - g0) * b0
    t1 = (1.0 - g1) * b1

    oa = jnp.concatenate([oa_s[0], oa_s[1]], axis=0).astype(BF16)
    acc = jnp.zeros((16, DM), F32)
    for gi in range(len(WO_GROUPS)):
        for _, cp in wo_tiles(gi):
            cp.wait()
        for hd0 in WO_GROUPS[gi]:
            for half in range(2):
                hd = half * 16 + hd0
                acc = acc + jnp.dot(oa[:, hd * DH:(hd + 1) * DH],
                                    wo_v[hd * DH:(hd + 1) * DH, :],
                                    preferred_element_type=F32)
    a_out = acc.astype(BF16).astype(F32)
    r0 = g0 * a_out[0:1, :] + t0
    r1 = g1 * a_out[8:9, :] + t1
    o_ref[...] = jnp.concatenate([r0, r1], axis=0).astype(o_ref.dtype)


@jax.jit
def pallas_gated_mix__mha_block_cached__compressed_kv_cla__decode_kernel(
    A_x: jax.Array,
    A_k_cache: jax.Array,
    A_v_cache: jax.Array,
    A_wq: jax.Array,
    A_wo: jax.Array,
    B_x: jax.Array,
    B_c_kv: jax.Array,
    B_w_q: jax.Array,
    B_w_uk: jax.Array,
    B_w_uv: jax.Array,
    B_w_o: jax.Array,
    gate_w: jax.Array,
):
    del B_x
    k2 = A_k_cache.reshape(NBH * SK, DH)
    v2 = A_v_cache.reshape(NBH * SK, DH)
    ckv2 = B_c_kv.reshape(NB * SK, DM)
    bwq2 = B_w_q.reshape(DM * NH, DH)
    wuk2 = B_w_uk.reshape(DM * NH, DH)
    wuv2 = B_w_uv.reshape(DM * NH, DH)
    bwo2 = B_w_o.reshape(NH * DH, DM)

    any_spec = pl.BlockSpec(memory_space=pl.ANY)
    scratch = [
        pltpu.VMEM((NB, DM), BF16),
        pltpu.VMEM((DM,), BF16),
        pltpu.VMEM((NSLOT, SK, DH), BF16),
        pltpu.VMEM((NSLOT, SK, DH), BF16),
        pltpu.VMEM((DM, NH * DH), BF16),
        pltpu.VMEM((NH * DH, DM), BF16),
        pltpu.VMEM((NB * SK, DM), BF16),
        pltpu.VMEM((DM * NH, DH), BF16),
        pltpu.VMEM((DM * NH, DH), BF16),
        pltpu.VMEM((DM * NH, DH), BF16),
        pltpu.VMEM((NH * DH, DM), BF16),
        pltpu.VMEM((DM * NH // 2, DH), jnp.uint32),
        pltpu.VMEM((DM * NH // 2, DH), jnp.uint32),
        pltpu.VMEM((NB, 16, NH * DH), BF16),
        pltpu.VMEM((NB, 8, NH * DH), F32),
        pltpu.VMEM((NB, NH, DM), F32),
        pltpu.VMEM((NB, NH, SK), F32),
        pltpu.VMEM((NB, NH, 128), F32),
        pltpu.VMEM((NB, NH, 128), F32),
        pltpu.VMEM((NB, NH, DM), F32),
        pltpu.VMEM((16, DM), F32),
        pltpu.SemaphoreType.DMA((NSLOT * NGRP,)),
        pltpu.SemaphoreType.DMA((NSLOT * NGRP,)),
        pltpu.SemaphoreType.DMA((8,)),
        pltpu.SemaphoreType.DMA((len(WO_GROUPS),)),
    ]
    out = pl.pallas_call(
        _kernel,
        out_shape=jax.ShapeDtypeStruct((NB, DM), BF16),
        in_specs=[any_spec] * 11,
        out_specs=pl.BlockSpec(memory_space=pltpu.VMEM),
        scratch_shapes=scratch,
        compiler_params=pltpu.CompilerParams(vmem_limit_bytes=100 * 1024 * 1024),
    )(A_x.reshape(NB, DM), gate_w, k2, v2, A_wq, A_wo, ckv2, bwq2, wuk2, wuv2, bwo2)
    return out.reshape(NB, 1, DM)
```

```python
import jax
import jax.numpy as jnp
from jax import lax
import jax.experimental.pallas as pl
import jax.experimental.pallas.tpu as pltpu

NB = 2
NH = 32
SK = 8192
DH = 128
DM = 512
NBH = NB * NH

TR = 128
WR = 32
NT = 64
QT = 16
NGRP = NT // QT
GROWS = QT * TR
NXB = 8
NSLOT = 2
CK = 2048

WO_GROUPS = ((0, 4, 8, 12), (1, 5, 9, 13), (2, 6, 10, 14), (3, 7, 11), (15,))
WO_IN_LOOP = 3

S_BPRO = 10
S_BSC = 16
S_BPV = S_BSC + 8
S_BEPI = S_BPV + 9

F32 = jnp.float32
BF16 = jnp.bfloat16
NT_DIMS = (((1,), (1,)), ((), ()))


def _stream_order(i):
    return (i % 4) * 16 + i // 4


def _kernel(x_hbm, gate_hbm, k_hbm, v_hbm, wq_hbm, wo_hbm, ckv_hbm, bwq_hbm, wuk_hbm,
            wuv_hbm, bwo_hbm, o_ref,
            x_v, gate_v, kbuf, vbuf, wq_v, wo_v, ckv_v, bwq_v, wuk_v, wuv_v, bwo_v,
            ua_s, ub_s, qa_s, oa_s, qabs_s, s_s, m_s, l_s, acc_s, outb_s,
            ksem, vsem, wsem):
    scale = DH ** -0.5

    def kv_tile(src, dst, sem, item, slot, grp, u):
        i = grp * QT + u
        return pltpu.make_async_copy(
            src.at[pl.ds(pl.multiple_of(item * SK + _stream_order(i) * TR, TR), TR)],
            dst.at[slot, pl.ds(i * TR, TR)],
            sem.at[grp])

    def issue_kv_group(item, grp):
        slot = item & (NSLOT - 1)
        for u in range(QT):
            kv_tile(k_hbm, kbuf, ksem, item, slot, grp, u).start(priority=0)
            kv_tile(v_hbm, vbuf, vsem, item, slot, grp, u).start(priority=1)

    def wait_kv_group(item, grp):
        slot = item & (NSLOT - 1)
        kb = kbuf.at[slot, pl.ds(grp * GROWS, GROWS)]
        vb = vbuf.at[slot, pl.ds(grp * GROWS, GROWS)]
        pltpu.make_async_copy(kb, kb, ksem.at[grp]).wait()
        pltpu.make_async_copy(vb, vb, vsem.at[grp]).wait()

    def rows_tile(src, dst, sem, rows, base, t):
        r0 = pl.multiple_of(base + t * rows, rows)
        return pltpu.make_async_copy(src.at[pl.ds(r0, rows)], dst.at[pl.ds(r0, rows)], sem)

    def issue_b_group(sx, grp):
        def pairs(src, dst, base0, base1, rows, sem):
            for u in range(QT):
                t = _stream_order(grp * QT + u)
                rows_tile(src, dst, sem, rows, base0, t).start(priority=0)
                rows_tile(src, dst, sem, rows, base1, t).start(priority=1)

        @pl.when(sx == 0)
        def _():
            pairs(bwq_hbm, bwq_v, 0, NT * TR, TR, wsem.at[0])

        @pl.when(sx == 1)
        def _():
            pairs(wuk_hbm, wuk_v, 0, NT * TR, TR, wsem.at[1])

        @pl.when(jnp.logical_and(sx >= 2, sx < 6))
        def _():
            base = pl.multiple_of((sx - 2) * CK, CK)
            pairs(ckv_hbm, ckv_v, base, SK + base, WR, wsem.at[2])

        @pl.when(sx == 6)
        def _():
            pairs(wuv_hbm, wuv_v, 0, NT * TR, TR, wsem.at[3])

        @pl.when(sx == 7)
        def _():
            pairs(bwo_hbm, bwo_v, 0, NT * WR, WR, wsem.at[4])

    def issue_wq():
        def tile(half, t):
            r0 = pl.multiple_of(half * 256 + (t >> 1) * 8, 8)
            c0 = pl.multiple_of((t & 1) * 2048, 2048)
            return pltpu.make_async_copy(
                wq_hbm.at[pl.ds(r0, 8), pl.ds(c0, 2048)],
                wq_v.at[pl.ds(r0, 8), pl.ds(c0, 2048)], wsem.at[5])

        def body(i, c):
            t = (i & 3) * 16 + (i >> 2)
            tile(0, t).start(priority=0)
            tile(1, t).start(priority=1)
            return c
        lax.fori_loop(0, NT, body, 0, unroll=4)

    def wo_tiles(gi):
        out = []
        for p in range(DH // WR):
            for hd in WO_GROUPS[gi]:
                for half in range(2):
                    r0 = (half * 16 + hd) * DH + p * WR
                    out.append((half, pltpu.make_async_copy(
                        wo_hbm.at[pl.ds(r0, WR)], wo_v.at[pl.ds(r0, WR)], wsem.at[gi])))
        return out

    def issue_wo_group(gi):
        for half, cp in wo_tiles(gi):
            cp.start(priority=half)

    def wait_full(buf, sem):
        pltpu.make_async_copy(buf, buf, sem).wait()

    x_cp = pltpu.make_async_copy(x_hbm, x_v, wsem.at[6])
    g_cp = pltpu.make_async_copy(gate_hbm, gate_v, wsem.at[6])
    x_cp.start()
    g_cp.start()
    issue_wq()
    for grp in range(NGRP):
        issue_kv_group(0, grp)

    outb_s[...] = jnp.zeros_like(outb_s)

    x_cp.wait()
    g_cp.wait()
    x2 = x_v[...].astype(F32)
    xf = jnp.concatenate([jnp.broadcast_to(x2[0:1], (8, DM)),
                          jnp.broadcast_to(x2[1:2], (8, DM))], axis=0)
    xb = xf.astype(BF16)
    gate = gate_v[...].astype(F32).reshape(1, DM)
    g = jax.nn.sigmoid(jnp.sum(xf * gate, axis=-1, keepdims=True))

    wait_full(wq_v, wsem.at[5])
    qa = jnp.dot(xb, wq_v[...], preferred_element_type=F32).astype(BF16)
    qa_s[0] = jnp.concatenate([qa[0:8], qa[0:8]], axis=0)
    qa_s[1] = jnp.concatenate([qa[8:16], qa[8:16]], axis=0)

    def to_words(w_v, u_s):
        def body(i, c):
            x = w_v[pl.ds(pl.multiple_of(i * 1024, 1024), 1024), :]
            u_s[pl.ds(pl.multiple_of(i * 512, 512), 512), :] = pltpu.bitcast(x, jnp.uint32)
            return c
        lax.fori_loop(0, DM * NH // 1024, body, 0)

    def deinterleave(u_s, j):
        u = u_s[pl.ds(j, DM, stride=NH // 2), :]
        lo = pltpu.bitcast(u << 16, F32).astype(BF16)
        hi = pltpu.bitcast(u & jnp.uint32(0xFFFF0000), F32).astype(BF16)
        return lo, hi

    def b_queries(grp):
        row = lax.broadcasted_iota(jnp.int32, (16, DH), 0) % 8
        tot = None
        for j in range(4 * grp, 4 * grp + 4):
            wq_pair = deinterleave(ua_s, j)
            wk_pair = deinterleave(ub_s, j)
            for e in range(2):
                q = jnp.dot(xb, wq_pair[e], preferred_element_type=F32).astype(BF16)
                q = jnp.where(row == (2 * j + e) % 8, q, jnp.zeros_like(q))
                qabs = lax.dot_general(q, wk_pair[e], NT_DIMS, preferred_element_type=F32)
                tot = qabs if tot is None else tot + qabs
        qabs_s[0, 8 * grp:8 * grp + 8, :] = tot[0:8]
        qabs_s[1, 8 * grp:8 * grp + 8, :] = tot[8:16]

    def b_scores(b, j):
        q = qabs_s[b].astype(BF16)
        c = ckv_v[pl.ds(pl.multiple_of(b * SK + j * CK, CK), CK), :]
        s = lax.dot_general(q, c, NT_DIMS, preferred_element_type=F32)
        s_s[b, :, pl.ds(pl.multiple_of(j * CK, CK), CK)] = s
        mx = jnp.broadcast_to(jnp.max(s, axis=-1, keepdims=True), (NH, 128))

        @pl.when(j == 0)
        def _():
            m_s[b] = mx

        @pl.when(j > 0)
        def _():
            m_s[b] = jnp.maximum(m_s[b], mx)

    def b_context(b, j):
        c = ckv_v[pl.ds(pl.multiple_of(b * SK + j * CK, CK), CK), :]
        s = s_s[b, :, pl.ds(pl.multiple_of(j * CK, CK), CK)]
        p = jnp.exp((s - m_s[b][:, 0:1]) * scale)
        ls = jnp.broadcast_to(jnp.sum(p, axis=-1, keepdims=True), (NH, 128))
        pv = jnp.dot(p.astype(BF16), c, preferred_element_type=F32)

        @pl.when(j == 0)
        def _():
            l_s[b] = ls
            acc_s[b] = pv

        @pl.when(j > 0)
        def _():
            l_s[b] = l_s[b] + ls
            acc_s[b] = acc_s[b] + pv

    def b_normalize():
        for b in range(NB):
            acc_s[b] = acc_s[b] / l_s[b][:, 0:1]

    def b_output(grp):
        row = lax.broadcasted_iota(jnp.int32, (16, DH), 0) % 8
        lhs = jnp.concatenate([acc_s[0, 8 * grp:8 * grp + 8, :],
                               acc_s[1, 8 * grp:8 * grp + 8, :]], axis=0).astype(BF16)
        tot = None
        for j in range(4 * grp, 4 * grp + 4):
            wv_pair = deinterleave(ua_s, j)
            for e in range(2):
                h = 2 * j + e
                ctx = jnp.dot(lhs, wv_pair[e], preferred_element_type=F32).astype(BF16)
                ctx = jnp.where(row == h % 8, ctx, jnp.zeros_like(ctx))
                part = jnp.dot(ctx, bwo_v[h * DH:(h + 1) * DH, :], preferred_element_type=F32)
                tot = part if tot is None else tot + part
        outb_s[...] += tot

    def b_work(s):
        @pl.when(s == S_BPRO - 2)
        def _():
            wait_full(bwq_v, wsem.at[0])
            to_words(bwq_v, ua_s)

        @pl.when(s == S_BPRO - 1)
        def _():
            wait_full(wuk_v, wsem.at[1])
            to_words(wuk_v, ub_s)

        for grp in range(4):
            pl.when(s == S_BPRO + grp)(lambda grp=grp: b_queries(grp))

        @pl.when(s == S_BSC)
        def _():
            wait_full(ckv_v, wsem.at[2])

        @pl.when(jnp.logical_and(s >= S_BSC, s < S_BPV))
        def _():
            i = s - S_BSC
            b_scores(i >> 2, i & 3)

        @pl.when(jnp.logical_and(s >= S_BPV, s < S_BPV + 8))
        def _():
            i = s - S_BPV
            b_context(i >> 2, i & 3)

        @pl.when(s == S_BEPI - 1)
        def _():
            wait_full(wuv_v, wsem.at[3])
            to_words(wuv_v, ua_s)

        @pl.when(s == S_BEPI)
        def _():
            wait_full(bwo_v, wsem.at[4])
            b_normalize()

        for grp in range(4):
            pl.when(s == S_BEPI + grp)(lambda grp=grp: b_output(grp))

    def a_item(s):
        b = s >> 5
        h = s & (NH - 1)
        slot = s & (NSLOT - 1)
        c0 = pl.multiple_of(h * DH, DH)
        q = qa_s[b, :, pl.ds(c0, DH)]
        sc = lax.dot_general(q, kbuf[slot], NT_DIMS, preferred_element_type=F32)
        m = jnp.max(sc, axis=-1, keepdims=True)
        p = jnp.exp((sc - m) * scale)
        l = jnp.sum(p, axis=-1, keepdims=True)
        o = jnp.dot(p.astype(BF16), vbuf[slot], preferred_element_type=F32)
        oa_s[b, :, pl.ds(c0, DH)] = (o / l)[0:8, :]

    def step(s, carry):
        nxt = s + 1
        has_b = s < NXB
        for grp in range(NGRP):
            wait_kv_group(s, grp)

            @pl.when(has_b)
            def _():
                issue_b_group(s, grp)

            @pl.when(jnp.logical_and(jnp.logical_not(has_b), nxt < NBH))
            def _():
                issue_kv_group(nxt, grp)

            if grp < WO_IN_LOOP:
                @pl.when(nxt == NBH)
                def _():
                    issue_wo_group(grp)

            if grp == 0:
                b_work(s)

        a_item(s)

        @pl.when(has_b)
        def _():
            for grp in range(NGRP):
                issue_kv_group(nxt, grp)
        return carry

    lax.fori_loop(0, NBH, step, 0)

    for gi in range(WO_IN_LOOP, len(WO_GROUPS)):
        issue_wo_group(gi)

    ob = outb_s[...]
    b0 = jnp.sum(ob[0:8], axis=0, keepdims=True).astype(BF16).astype(F32)
    b1 = jnp.sum(ob[8:16], axis=0, keepdims=True).astype(BF16).astype(F32)
    g0 = g[0:1, :]
    g1 = g[8:9, :]
    t0 = (1.0 - g0) * b0
    t1 = (1.0 - g1) * b1

    oa = jnp.concatenate([oa_s[0], oa_s[1]], axis=0).astype(BF16)
    acc = jnp.zeros((16, DM), F32)
    for gi in range(len(WO_GROUPS)):
        for _, cp in wo_tiles(gi):
            cp.wait()
        for hd0 in WO_GROUPS[gi]:
            for half in range(2):
                hd = half * 16 + hd0
                acc = acc + jnp.dot(oa[:, hd * DH:(hd + 1) * DH],
                                    wo_v[hd * DH:(hd + 1) * DH, :],
                                    preferred_element_type=F32)
    a_out = acc.astype(BF16).astype(F32)
    r0 = g0 * a_out[0:1, :] + t0
    r1 = g1 * a_out[8:9, :] + t1
    o_ref[...] = jnp.concatenate([r0, r1], axis=0).astype(o_ref.dtype)


@jax.jit
def pallas_gated_mix__mha_block_cached__compressed_kv_cla__decode_kernel(
    A_x: jax.Array,
    A_k_cache: jax.Array,
    A_v_cache: jax.Array,
    A_wq: jax.Array,
    A_wo: jax.Array,
    B_x: jax.Array,
    B_c_kv: jax.Array,
    B_w_q: jax.Array,
    B_w_uk: jax.Array,
    B_w_uv: jax.Array,
    B_w_o: jax.Array,
    gate_w: jax.Array,
):
    del B_x
    k2 = A_k_cache.reshape(NBH * SK, DH)
    v2 = A_v_cache.reshape(NBH * SK, DH)
    ckv2 = B_c_kv.reshape(NB * SK, DM)
    bwq2 = B_w_q.reshape(DM * NH, DH)
    wuk2 = B_w_uk.reshape(DM * NH, DH)
    wuv2 = B_w_uv.reshape(DM * NH, DH)
    bwo2 = B_w_o.reshape(NH * DH, DM)

    any_spec = pl.BlockSpec(memory_space=pl.ANY)
    scratch = [
        pltpu.VMEM((NB, DM), BF16),
        pltpu.VMEM((DM,), BF16),
        pltpu.VMEM((NSLOT, SK, DH), BF16),
        pltpu.VMEM((NSLOT, SK, DH), BF16),
        pltpu.VMEM((DM, NH * DH), BF16),
        pltpu.VMEM((NH * DH, DM), BF16),
        pltpu.VMEM((NB * SK, DM), BF16),
        pltpu.VMEM((DM * NH, DH), BF16),
        pltpu.VMEM((DM * NH, DH), BF16),
        pltpu.VMEM((DM * NH, DH), BF16),
        pltpu.VMEM((NH * DH, DM), BF16),
        pltpu.VMEM((DM * NH // 2, DH), jnp.uint32),
        pltpu.VMEM((DM * NH // 2, DH), jnp.uint32),
        pltpu.VMEM((NB, 16, NH * DH), BF16),
        pltpu.VMEM((NB, 8, NH * DH), F32),
        pltpu.VMEM((NB, NH, DM), F32),
        pltpu.VMEM((NB, NH, SK), F32),
        pltpu.VMEM((NB, NH, 128), F32),
        pltpu.VMEM((NB, NH, 128), F32),
        pltpu.VMEM((NB, NH, DM), F32),
        pltpu.VMEM((16, DM), F32),
        pltpu.SemaphoreType.DMA((NGRP,)),
        pltpu.SemaphoreType.DMA((NGRP,)),
        pltpu.SemaphoreType.DMA((7,)),
    ]
    out = pl.pallas_call(
        _kernel,
        out_shape=jax.ShapeDtypeStruct((NB, DM), BF16),
        in_specs=[any_spec] * 11,
        out_specs=pl.BlockSpec(memory_space=pltpu.VMEM),
        scratch_shapes=scratch,
        compiler_params=pltpu.CompilerParams(vmem_limit_bytes=100 * 1024 * 1024),
    )(A_x.reshape(NB, DM), gate_w, k2, v2, A_wq, A_wo, ckv2, bwq2, wuk2, wuv2, bwo2)
    return out.reshape(NB, 1, DM)
```

```python
import jax
import jax.numpy as jnp
from jax import lax
import jax.experimental.pallas as pl
import jax.experimental.pallas.tpu as pltpu

NB = 2
NH = 32
SK = 8192
DH = 128
DM = 512
NBH = NB * NH

TR = 128
WR = 32
NT = 64
QT = 16
NGRP = NT // QT
GROWS = QT * TR
NXB = 8
NSLOT = 2
CK = 2048

WO_GROUPS = ((0, 4, 8, 12), (1, 5, 9, 13), (2, 6, 10, 14), (3, 7, 11), (15,))
WO_IN_LOOP = 3

S_BPRO = 10
S_BSC = 16
S_BPV = S_BSC + 8
S_BEPI = S_BPV + 9

F32 = jnp.float32
BF16 = jnp.bfloat16
NT_DIMS = (((1,), (1,)), ((), ()))


def _stream_order(i):
    return (i % 4) * 16 + i // 4


def _kernel(x_hbm, gate_hbm, k_hbm, v_hbm, wq_hbm, wo_hbm, ckv_hbm, bwq_hbm, wuk_hbm,
            wuv_hbm, bwo_hbm, o_ref,
            x_v, gate_v, kbuf, vbuf, wq_v, wo_v, ckv_v, bwq_v, wuk_v, wuv_v, bwo_v,
            ua_s, ub_s, qa_s, oa_s, qabs_s, s_s, m_s, l_s, acc_s, outb_s,
            ksem, vsem, wsem):
    scale = DH ** -0.5

    def kv_tile(src, dst, sem, item, slot, grp, u):
        i = grp * QT + u
        return pltpu.make_async_copy(
            src.at[pl.ds(pl.multiple_of(item * SK + _stream_order(i) * TR, TR), TR)],
            dst.at[slot, pl.ds(i * TR, TR)],
            sem.at[grp])

    def issue_kv_group(item, grp):
        slot = item & (NSLOT - 1)
        for u in range(QT):
            kv_tile(k_hbm, kbuf, ksem, item, slot, grp, u).start(priority=0)
            kv_tile(v_hbm, vbuf, vsem, item, slot, grp, u).start(priority=1)

    def wait_kv_group(item, grp):
        slot = item & (NSLOT - 1)
        kb = kbuf.at[slot, pl.ds(grp * GROWS, GROWS)]
        vb = vbuf.at[slot, pl.ds(grp * GROWS, GROWS)]
        pltpu.make_async_copy(kb, kb, ksem.at[grp]).wait()
        pltpu.make_async_copy(vb, vb, vsem.at[grp]).wait()

    def rows_tile(src, dst, sem, rows, base, t):
        r0 = pl.multiple_of(base + t * rows, rows)
        return pltpu.make_async_copy(src.at[pl.ds(r0, rows)], dst.at[pl.ds(r0, rows)], sem)

    def issue_b_group(sx, grp):
        def pairs(src, dst, base0, base1, rows, sem):
            for u in range(QT):
                t = _stream_order(grp * QT + u)
                rows_tile(src, dst, sem, rows, base0, t).start(priority=0)
                rows_tile(src, dst, sem, rows, base1, t).start(priority=1)

        @pl.when(sx == 0)
        def _():
            pairs(bwq_hbm, bwq_v, 0, NT * TR, TR, wsem.at[0])

        @pl.when(sx == 1)
        def _():
            pairs(wuk_hbm, wuk_v, 0, NT * TR, TR, wsem.at[1])

        @pl.when(jnp.logical_and(sx >= 2, sx < 6))
        def _():
            base = pl.multiple_of((sx - 2) * CK, CK)
            pairs(ckv_hbm, ckv_v, base, SK + base, WR, wsem.at[2])

        @pl.when(sx == 6)
        def _():
            pairs(wuv_hbm, wuv_v, 0, NT * TR, TR, wsem.at[3])

        @pl.when(sx == 7)
        def _():
            pairs(bwo_hbm, bwo_v, 0, NT * WR, WR, wsem.at[4])

    def issue_wq():
        def tile(half, t):
            r0 = pl.multiple_of(half * 256 + (t >> 1) * 8, 8)
            c0 = pl.multiple_of((t & 1) * 2048, 2048)
            return pltpu.make_async_copy(
                wq_hbm.at[pl.ds(r0, 8), pl.ds(c0, 2048)],
                wq_v.at[pl.ds(r0, 8), pl.ds(c0, 2048)], wsem.at[2])

        def body(i, c):
            t = (i & 3) * 16 + (i >> 2)
            tile(0, t).start(priority=0)
            tile(1, t).start(priority=1)
            return c
        lax.fori_loop(0, NT, body, 0, unroll=4)

    def wo_tiles(gi):
        out = []
        for p in range(DH // WR):
            for hd in WO_GROUPS[gi]:
                for half in range(2):
                    r0 = (half * 16 + hd) * DH + p * WR
                    out.append((half, pltpu.make_async_copy(
                        wo_hbm.at[pl.ds(r0, WR)], wo_v.at[pl.ds(r0, WR)], wsem.at[gi])))
        return out

    def issue_wo_group(gi):
        for half, cp in wo_tiles(gi):
            cp.start(priority=half)

    def wait_full(buf, sem):
        pltpu.make_async_copy(buf, buf, sem).wait()

    x_cp = pltpu.make_async_copy(x_hbm, x_v, wsem.at[0])
    g_cp = pltpu.make_async_copy(gate_hbm, gate_v, wsem.at[1])
    x_cp.start()
    g_cp.start()
    issue_wq()
    for grp in range(NGRP):
        issue_kv_group(0, grp)

    outb_s[...] = jnp.zeros_like(outb_s)

    x_cp.wait()
    g_cp.wait()
    x2 = x_v[...].astype(F32)
    xf = jnp.concatenate([jnp.broadcast_to(x2[0:1], (8, DM)),
                          jnp.broadcast_to(x2[1:2], (8, DM))], axis=0)
    xb = xf.astype(BF16)
    gate = gate_v[...].astype(F32).reshape(1, DM)
    g = jax.nn.sigmoid(jnp.sum(xf * gate, axis=-1, keepdims=True))

    wait_full(wq_v, wsem.at[2])
    qa = jnp.dot(xb, wq_v[...], preferred_element_type=F32).astype(BF16)
    qa_s[0] = jnp.concatenate([qa[0:8], qa[0:8]], axis=0)
    qa_s[1] = jnp.concatenate([qa[8:16], qa[8:16]], axis=0)

    def to_words(w_v, u_s):
        def body(i, c):
            x = w_v[pl.ds(pl.multiple_of(i * 1024, 1024), 1024), :]
            u_s[pl.ds(pl.multiple_of(i * 512, 512), 512), :] = pltpu.bitcast(x, jnp.uint32)
            return c
        lax.fori_loop(0, DM * NH // 1024, body, 0)

    def deinterleave(u_s, j):
        u = u_s[pl.ds(j, DM, stride=NH // 2), :]
        lo = pltpu.bitcast(u << 16, F32).astype(BF16)
        hi = pltpu.bitcast(u & jnp.uint32(0xFFFF0000), F32).astype(BF16)
        return lo, hi

    def b_queries(grp):
        row = lax.broadcasted_iota(jnp.int32, (16, DH), 0) % 8
        tot = None
        for j in range(4 * grp, 4 * grp + 4):
            wq_pair = deinterleave(ua_s, j)
            wk_pair = deinterleave(ub_s, j)
            for e in range(2):
                q = jnp.dot(xb, wq_pair[e], preferred_element_type=F32).astype(BF16)
                q = jnp.where(row == (2 * j + e) % 8, q, jnp.zeros_like(q))
                qabs = lax.dot_general(q, wk_pair[e], NT_DIMS, preferred_element_type=F32)
                tot = qabs if tot is None else tot + qabs
        qabs_s[0, 8 * grp:8 * grp + 8, :] = tot[0:8]
        qabs_s[1, 8 * grp:8 * grp + 8, :] = tot[8:16]

    def b_scores(b, j):
        q = qabs_s[b].astype(BF16)
        c = ckv_v[pl.ds(pl.multiple_of(b * SK + j * CK, CK), CK), :]
        s = lax.dot_general(q, c, NT_DIMS, preferred_element_type=F32)
        s_s[b, :, pl.ds(pl.multiple_of(j * CK, CK), CK)] = s
        mx = jnp.broadcast_to(jnp.max(s, axis=-1, keepdims=True), (NH, 128))

        @pl.when(j == 0)
        def _():
            m_s[b] = mx

        @pl.when(j > 0)
        def _():
            m_s[b] = jnp.maximum(m_s[b], mx)

    def b_context(b, j):
        c = ckv_v[pl.ds(pl.multiple_of(b * SK + j * CK, CK), CK), :]
        s = s_s[b, :, pl.ds(pl.multiple_of(j * CK, CK), CK)]
        p = jnp.exp((s - m_s[b][:, 0:1]) * scale)
        ls = jnp.broadcast_to(jnp.sum(p, axis=-1, keepdims=True), (NH, 128))
        pv = jnp.dot(p.astype(BF16), c, preferred_element_type=F32)

        @pl.when(j == 0)
        def _():
            l_s[b] = ls
            acc_s[b] = pv

        @pl.when(j > 0)
        def _():
            l_s[b] = l_s[b] + ls
            acc_s[b] = acc_s[b] + pv

    def b_normalize():
        for b in range(NB):
            acc_s[b] = acc_s[b] / l_s[b][:, 0:1]

    def b_output(grp):
        row = lax.broadcasted_iota(jnp.int32, (16, DH), 0) % 8
        lhs = jnp.concatenate([acc_s[0, 8 * grp:8 * grp + 8, :],
                               acc_s[1, 8 * grp:8 * grp + 8, :]], axis=0).astype(BF16)
        tot = None
        for j in range(4 * grp, 4 * grp + 4):
            wv_pair = deinterleave(ua_s, j)
            for e in range(2):
                h = 2 * j + e
                ctx = jnp.dot(lhs, wv_pair[e], preferred_element_type=F32).astype(BF16)
                ctx = jnp.where(row == h % 8, ctx, jnp.zeros_like(ctx))
                part = jnp.dot(ctx, bwo_v[h * DH:(h + 1) * DH, :], preferred_element_type=F32)
                tot = part if tot is None else tot + part
        outb_s[...] += tot

    def b_work(s):
        @pl.when(s == S_BPRO - 2)
        def _():
            wait_full(bwq_v, wsem.at[0])
            to_words(bwq_v, ua_s)

        @pl.when(s == S_BPRO - 1)
        def _():
            wait_full(wuk_v, wsem.at[1])
            to_words(wuk_v, ub_s)

        for grp in range(4):
            pl.when(s == S_BPRO + grp)(lambda grp=grp: b_queries(grp))

        @pl.when(s == S_BSC)
        def _():
            wait_full(ckv_v, wsem.at[2])

        @pl.when(jnp.logical_and(s >= S_BSC, s < S_BPV))
        def _():
            i = s - S_BSC
            b_scores(i >> 2, i & 3)

        @pl.when(jnp.logical_and(s >= S_BPV, s < S_BPV + 8))
        def _():
            i = s - S_BPV
            b_context(i >> 2, i & 3)

        @pl.when(s == S_BEPI - 1)
        def _():
            wait_full(wuv_v, wsem.at[3])
            to_words(wuv_v, ua_s)

        @pl.when(s == S_BEPI)
        def _():
            wait_full(bwo_v, wsem.at[4])
            b_normalize()

        for grp in range(4):
            pl.when(s == S_BEPI + grp)(lambda grp=grp: b_output(grp))

    def a_item(s):
        b = s >> 5
        h = s & (NH - 1)
        slot = s & (NSLOT - 1)
        c0 = pl.multiple_of(h * DH, DH)
        q = qa_s[b, :, pl.ds(c0, DH)]
        sc = lax.dot_general(q, kbuf[slot], NT_DIMS, preferred_element_type=F32)
        m = jnp.max(sc, axis=-1, keepdims=True)
        p = jnp.exp((sc - m) * scale)
        l = jnp.sum(p, axis=-1, keepdims=True)
        o = jnp.dot(p.astype(BF16), vbuf[slot], preferred_element_type=F32)
        oa_s[b, :, pl.ds(c0, DH)] = (o / l)[0:8, :]

    def step(s, carry):
        nxt = s + 1
        has_b = s < NXB
        for grp in range(NGRP):
            wait_kv_group(s, grp)

            @pl.when(has_b)
            def _():
                issue_b_group(s, grp)

            @pl.when(jnp.logical_and(jnp.logical_not(has_b), nxt < NBH))
            def _():
                issue_kv_group(nxt, grp)

            if grp < WO_IN_LOOP:
                @pl.when(nxt == NBH)
                def _():
                    issue_wo_group(grp)

            if grp == 0:
                b_work(s)

        a_item(s)

        @pl.when(has_b)
        def _():
            for grp in range(NGRP):
                issue_kv_group(nxt, grp)
        return carry

    lax.fori_loop(0, NBH, step, 0)

    for gi in range(WO_IN_LOOP, len(WO_GROUPS)):
        issue_wo_group(gi)

    ob = outb_s[...]
    b0 = jnp.sum(ob[0:8], axis=0, keepdims=True).astype(BF16).astype(F32)
    b1 = jnp.sum(ob[8:16], axis=0, keepdims=True).astype(BF16).astype(F32)
    g0 = g[0:1, :]
    g1 = g[8:9, :]
    t0 = (1.0 - g0) * b0
    t1 = (1.0 - g1) * b1

    oa = jnp.concatenate([oa_s[0], oa_s[1]], axis=0).astype(BF16)
    acc = jnp.zeros((16, DM), F32)
    for gi in range(len(WO_GROUPS)):
        for _, cp in wo_tiles(gi):
            cp.wait()
        for hd0 in WO_GROUPS[gi]:
            for half in range(2):
                hd = half * 16 + hd0
                acc = acc + jnp.dot(oa[:, hd * DH:(hd + 1) * DH],
                                    wo_v[hd * DH:(hd + 1) * DH, :],
                                    preferred_element_type=F32)
    a_out = acc.astype(BF16).astype(F32)
    r0 = g0 * a_out[0:1, :] + t0
    r1 = g1 * a_out[8:9, :] + t1
    o_ref[...] = jnp.concatenate([r0, r1], axis=0).astype(o_ref.dtype)


@jax.jit
def pallas_gated_mix__mha_block_cached__compressed_kv_cla__decode_kernel(
    A_x: jax.Array,
    A_k_cache: jax.Array,
    A_v_cache: jax.Array,
    A_wq: jax.Array,
    A_wo: jax.Array,
    B_x: jax.Array,
    B_c_kv: jax.Array,
    B_w_q: jax.Array,
    B_w_uk: jax.Array,
    B_w_uv: jax.Array,
    B_w_o: jax.Array,
    gate_w: jax.Array,
):
    del B_x
    k2 = A_k_cache.reshape(NBH * SK, DH)
    v2 = A_v_cache.reshape(NBH * SK, DH)
    ckv2 = B_c_kv.reshape(NB * SK, DM)
    bwq2 = B_w_q.reshape(DM * NH, DH)
    wuk2 = B_w_uk.reshape(DM * NH, DH)
    wuv2 = B_w_uv.reshape(DM * NH, DH)
    bwo2 = B_w_o.reshape(NH * DH, DM)

    any_spec = pl.BlockSpec(memory_space=pl.ANY)
    scratch = [
        pltpu.VMEM((NB, DM), BF16),
        pltpu.VMEM((DM,), BF16),
        pltpu.VMEM((NSLOT, SK, DH), BF16),
        pltpu.VMEM((NSLOT, SK, DH), BF16),
        pltpu.VMEM((DM, NH * DH), BF16),
        pltpu.VMEM((NH * DH, DM), BF16),
        pltpu.VMEM((NB * SK, DM), BF16),
        pltpu.VMEM((DM * NH, DH), BF16),
        pltpu.VMEM((DM * NH, DH), BF16),
        pltpu.VMEM((DM * NH, DH), BF16),
        pltpu.VMEM((NH * DH, DM), BF16),
        pltpu.VMEM((DM * NH // 2 + 16, DH), jnp.uint32),
        pltpu.VMEM((DM * NH // 2 + 16, DH), jnp.uint32),
        pltpu.VMEM((NB, 16, NH * DH), BF16),
        pltpu.VMEM((NB, 8, NH * DH), F32),
        pltpu.VMEM((NB, NH, DM), F32),
        pltpu.VMEM((NB, NH, SK), F32),
        pltpu.VMEM((NB, NH, 128), F32),
        pltpu.VMEM((NB, NH, 128), F32),
        pltpu.VMEM((NB, NH, DM), F32),
        pltpu.VMEM((16, DM), F32),
        pltpu.SemaphoreType.DMA((NGRP,)),
        pltpu.SemaphoreType.DMA((NGRP,)),
        pltpu.SemaphoreType.DMA((5,)),
    ]
    out = pl.pallas_call(
        _kernel,
        out_shape=jax.ShapeDtypeStruct((NB, DM), BF16),
        in_specs=[any_spec] * 11,
        out_specs=pl.BlockSpec(memory_space=pltpu.VMEM),
        scratch_shapes=scratch,
        compiler_params=pltpu.CompilerParams(vmem_limit_bytes=100 * 1024 * 1024),
    )(A_x.reshape(NB, DM), gate_w, k2, v2, A_wq, A_wo, ckv2, bwq2, wuk2, wuv2, bwo2)
    return out.reshape(NB, 1, DM)
```

```python
import jax
import jax.numpy as jnp
from jax import lax
import jax.experimental.pallas as pl
import jax.experimental.pallas.tpu as pltpu

NB = 2
NH = 32
SK = 8192
DH = 128
DM = 512
NBH = NB * NH

TR = 128
WR = 32
NT = 64
QT = 16
NGRP = NT // QT
GROWS = QT * TR
NXB = 8
NSLOT = 2
CK = 2048

WO_GROUPS = ((0, 4, 8, 12), (1, 5, 9, 13), (2, 6, 10, 14), (3, 7, 11), (15,))
WO_IN_LOOP = 3

S_BPRO = 10
S_BSC = 16
S_BPV = S_BSC + 8
S_BEPI = S_BPV + 9

F32 = jnp.float32
BF16 = jnp.bfloat16
NT_DIMS = (((1,), (1,)), ((), ()))


def _stream_order(i):
    return (i % 4) * 16 + i // 4


def _kernel(x_hbm, gate_hbm, k_hbm, v_hbm, wq_hbm, wo_hbm, ckv_hbm, bwq_hbm, wuk_hbm,
            wuv_hbm, bwo_hbm, o_ref,
            x_v, gate_v, kbuf, vbuf, wq_v, wo_v, ckv_v, bwq_v, wuk_v, wuv_v, bwo_v,
            ua_s, ub_s, qa_s, oa_s, qabs_s, s_s, m_s, l_s, acc_s, outb_s,
            ksem, vsem, wsem):
    scale = DH ** -0.5

    def kv_tile(src, dst, sem, item, slot, grp, u):
        i = grp * QT + u
        return pltpu.make_async_copy(
            src.at[pl.ds(pl.multiple_of(item * SK + _stream_order(i) * TR, TR), TR)],
            dst.at[slot, pl.ds(i * TR, TR)],
            sem.at[grp])

    def issue_kv_group(item, grp):
        slot = item & (NSLOT - 1)
        for u in range(QT):
            kv_tile(k_hbm, kbuf, ksem, item, slot, grp, u).start(priority=0)
            kv_tile(v_hbm, vbuf, vsem, item, slot, grp, u).start(priority=1)

    def wait_kv_group(item, grp):
        slot = item & (NSLOT - 1)
        kb = kbuf.at[slot, pl.ds(grp * GROWS, GROWS)]
        vb = vbuf.at[slot, pl.ds(grp * GROWS, GROWS)]
        pltpu.make_async_copy(kb, kb, ksem.at[grp]).wait()
        pltpu.make_async_copy(vb, vb, vsem.at[grp]).wait()

    def rows_tile(src, dst, sem, rows, base, t):
        r0 = pl.multiple_of(base + t * rows, rows)
        return pltpu.make_async_copy(src.at[pl.ds(r0, rows)], dst.at[pl.ds(r0, rows)], sem)

    def issue_b_group(sx, grp):
        def pairs(src, dst, base0, base1, rows, sem):
            for u in range(QT):
                t = _stream_order(grp * QT + u)
                rows_tile(src, dst, sem, rows, base0, t).start(priority=0)
                rows_tile(src, dst, sem, rows, base1, t).start(priority=1)

        @pl.when(sx == 0)
        def _():
            pairs(bwq_hbm, bwq_v, 0, NT * TR, TR, wsem.at[0])

        @pl.when(sx == 1)
        def _():
            pairs(wuk_hbm, wuk_v, 0, NT * TR, TR, wsem.at[1])

        @pl.when(jnp.logical_and(sx >= 2, sx < 6))
        def _():
            base = pl.multiple_of((sx - 2) * CK, CK)
            pairs(ckv_hbm, ckv_v, base, SK + base, WR, wsem.at[2])

        @pl.when(sx == 6)
        def _():
            pairs(wuv_hbm, wuv_v, 0, NT * TR, TR, wsem.at[3])

        @pl.when(sx == 7)
        def _():
            pairs(bwo_hbm, bwo_v, 0, NT * WR, WR, wsem.at[4])

    def issue_wq():
        def tile(half, t):
            r0 = pl.multiple_of(half * 256 + (t >> 1) * 8, 8)
            c0 = pl.multiple_of((t & 1) * 2048, 2048)
            return pltpu.make_async_copy(
                wq_hbm.at[pl.ds(r0, 8), pl.ds(c0, 2048)],
                wq_v.at[pl.ds(r0, 8), pl.ds(c0, 2048)], wsem.at[2])

        def body(i, c):
            t = (i & 3) * 16 + (i >> 2)
            tile(0, t).start(priority=0)
            tile(1, t).start(priority=1)
            return c
        lax.fori_loop(0, NT, body, 0, unroll=4)

    def wo_tiles(gi):
        out = []
        for p in range(DH // WR):
            for hd in WO_GROUPS[gi]:
                for half in range(2):
                    r0 = (half * 16 + hd) * DH + p * WR
                    out.append((half, pltpu.make_async_copy(
                        wo_hbm.at[pl.ds(r0, WR)], wo_v.at[pl.ds(r0, WR)], wsem.at[gi])))
        return out

    def issue_wo_group(gi):
        for half, cp in wo_tiles(gi):
            cp.start(priority=half)

    def wait_full(buf, sem):
        pltpu.make_async_copy(buf, buf, sem).wait()

    x_cp = pltpu.make_async_copy(x_hbm, x_v, wsem.at[0])
    g_cp = pltpu.make_async_copy(gate_hbm, gate_v, wsem.at[1])
    x_cp.start()
    g_cp.start()
    issue_wq()
    for grp in range(NGRP):
        issue_kv_group(0, grp)

    outb_s[...] = jnp.zeros_like(outb_s)

    x_cp.wait()
    g_cp.wait()
    x2 = x_v[...].astype(F32)
    xf = jnp.concatenate([jnp.broadcast_to(x2[0:1], (8, DM)),
                          jnp.broadcast_to(x2[1:2], (8, DM))], axis=0)
    xb = xf.astype(BF16)
    gate = gate_v[...].astype(F32).reshape(1, DM)
    g = jax.nn.sigmoid(jnp.sum(xf * gate, axis=-1, keepdims=True))

    wait_full(wq_v, wsem.at[2])
    qa = jnp.dot(xb, wq_v[...], preferred_element_type=F32).astype(BF16)
    qa_s[0] = jnp.concatenate([qa[0:8], qa[0:8]], axis=0)
    qa_s[1] = jnp.concatenate([qa[8:16], qa[8:16]], axis=0)

    def to_words(w_v, u_s):
        def body(i, c):
            x = w_v[pl.ds(pl.multiple_of(i * 1024, 1024), 1024), :]
            u_s[pl.ds(pl.multiple_of(i * 512, 512), 512), :] = pltpu.bitcast(x, jnp.uint32)
            return c
        lax.fori_loop(0, DM * NH // 1024, body, 0)

    def deinterleave(u_s, j):
        u = u_s[pl.ds(j, DM, stride=NH // 2), :]
        lo = pltpu.bitcast(u << 16, F32).astype(BF16)
        hi = pltpu.bitcast(u & jnp.uint32(0xFFFF0000), F32).astype(BF16)
        return lo, hi

    def b_queries(grp):
        row = lax.broadcasted_iota(jnp.int32, (16, DH), 0) % 8
        tot = None
        for j in range(4 * grp, 4 * grp + 4):
            wq_pair = deinterleave(ua_s, j)
            wk_pair = deinterleave(ub_s, j)
            for e in range(2):
                q = jnp.dot(xb, wq_pair[e], preferred_element_type=F32).astype(BF16)
                q = jnp.where(row == (2 * j + e) % 8, q, jnp.zeros_like(q))
                qabs = lax.dot_general(q, wk_pair[e], NT_DIMS, preferred_element_type=F32)
                tot = qabs if tot is None else tot + qabs
        qabs_s[0, 8 * grp:8 * grp + 8, :] = tot[0:8]
        qabs_s[1, 8 * grp:8 * grp + 8, :] = tot[8:16]

    def b_scores(b, j):
        q32 = qabs_s[b]
        q_hi = q32.astype(BF16)
        q_lo = (q32 - q_hi.astype(F32)).astype(BF16)
        q = jnp.concatenate([q_hi, q_lo], axis=0)
        c = ckv_v[pl.ds(pl.multiple_of(b * SK + j * CK, CK), CK), :]
        s2 = lax.dot_general(q, c, NT_DIMS, preferred_element_type=F32)
        s = s2[0:NH] + s2[NH:2 * NH]
        s_s[b, :, pl.ds(pl.multiple_of(j * CK, CK), CK)] = s
        mx = jnp.broadcast_to(jnp.max(s, axis=-1, keepdims=True), (NH, 128))

        @pl.when(j == 0)
        def _():
            m_s[b] = mx

        @pl.when(j > 0)
        def _():
            m_s[b] = jnp.maximum(m_s[b], mx)

    def b_context(b, j):
        c = ckv_v[pl.ds(pl.multiple_of(b * SK + j * CK, CK), CK), :]
        s = s_s[b, :, pl.ds(pl.multiple_of(j * CK, CK), CK)]
        p = jnp.exp((s - m_s[b][:, 0:1]) * scale)
        ls = jnp.broadcast_to(jnp.sum(p, axis=-1, keepdims=True), (NH, 128))
        pv = jnp.dot(p.astype(BF16), c, preferred_element_type=F32)

        @pl.when(j == 0)
        def _():
            l_s[b] = ls
            acc_s[b] = pv

        @pl.when(j > 0)
        def _():
            l_s[b] = l_s[b] + ls
            acc_s[b] = acc_s[b] + pv

    def b_normalize():
        for b in range(NB):
            acc_s[b] = acc_s[b] / l_s[b][:, 0:1]

    def b_output(grp):
        row = lax.broadcasted_iota(jnp.int32, (16, DH), 0) % 8
        lhs = jnp.concatenate([acc_s[0, 8 * grp:8 * grp + 8, :],
                               acc_s[1, 8 * grp:8 * grp + 8, :]], axis=0).astype(BF16)
        tot = None
        for j in range(4 * grp, 4 * grp + 4):
            wv_pair = deinterleave(ua_s, j)
            for e in range(2):
                h = 2 * j + e
                ctx = jnp.dot(lhs, wv_pair[e], preferred_element_type=F32).astype(BF16)
                ctx = jnp.where(row == h % 8, ctx, jnp.zeros_like(ctx))
                part = jnp.dot(ctx, bwo_v[h * DH:(h + 1) * DH, :], preferred_element_type=F32)
                tot = part if tot is None else tot + part
        outb_s[...] += tot

    def b_work(s):
        @pl.when(s == S_BPRO - 2)
        def _():
            wait_full(bwq_v, wsem.at[0])
            to_words(bwq_v, ua_s)

        @pl.when(s == S_BPRO - 1)
        def _():
            wait_full(wuk_v, wsem.at[1])
            to_words(wuk_v, ub_s)

        for grp in range(4):
            pl.when(s == S_BPRO + grp)(lambda grp=grp: b_queries(grp))

        @pl.when(s == S_BSC)
        def _():
            wait_full(ckv_v, wsem.at[2])

        @pl.when(jnp.logical_and(s >= S_BSC, s < S_BPV))
        def _():
            i = s - S_BSC
            b_scores(i >> 2, i & 3)

        @pl.when(jnp.logical_and(s >= S_BPV, s < S_BPV + 8))
        def _():
            i = s - S_BPV
            b_context(i >> 2, i & 3)

        @pl.when(s == S_BEPI - 1)
        def _():
            wait_full(wuv_v, wsem.at[3])
            to_words(wuv_v, ua_s)

        @pl.when(s == S_BEPI)
        def _():
            wait_full(bwo_v, wsem.at[4])
            b_normalize()

        for grp in range(4):
            pl.when(s == S_BEPI + grp)(lambda grp=grp: b_output(grp))

    def a_item(s):
        b = s >> 5
        h = s & (NH - 1)
        slot = s & (NSLOT - 1)
        c0 = pl.multiple_of(h * DH, DH)
        q = qa_s[b, :, pl.ds(c0, DH)]
        sc = lax.dot_general(q, kbuf[slot], NT_DIMS, preferred_element_type=F32)
        m = jnp.max(sc, axis=-1, keepdims=True)
        p = jnp.exp((sc - m) * scale)
        l = jnp.sum(p, axis=-1, keepdims=True)
        o = jnp.dot(p.astype(BF16), vbuf[slot], preferred_element_type=F32)
        oa_s[b, :, pl.ds(c0, DH)] = (o / l)[0:8, :]

    def step(s, carry):
        nxt = s + 1
        has_b = s < NXB
        for grp in range(NGRP):
            wait_kv_group(s, grp)

            @pl.when(has_b)
            def _():
                issue_b_group(s, grp)

            @pl.when(jnp.logical_and(jnp.logical_not(has_b), nxt < NBH))
            def _():
                issue_kv_group(nxt, grp)

            if grp < WO_IN_LOOP:
                @pl.when(nxt == NBH)
                def _():
                    issue_wo_group(grp)

            if grp == 0:
                b_work(s)

        a_item(s)

        @pl.when(has_b)
        def _():
            for grp in range(NGRP):
                issue_kv_group(nxt, grp)
        return carry

    lax.fori_loop(0, NBH, step, 0)

    for gi in range(WO_IN_LOOP, len(WO_GROUPS)):
        issue_wo_group(gi)

    ob = outb_s[...]
    b0 = jnp.sum(ob[0:8], axis=0, keepdims=True).astype(BF16).astype(F32)
    b1 = jnp.sum(ob[8:16], axis=0, keepdims=True).astype(BF16).astype(F32)
    g0 = g[0:1, :]
    g1 = g[8:9, :]
    t0 = (1.0 - g0) * b0
    t1 = (1.0 - g1) * b1

    oa = jnp.concatenate([oa_s[0], oa_s[1]], axis=0).astype(BF16)
    acc = jnp.zeros((16, DM), F32)
    for gi in range(len(WO_GROUPS)):
        for _, cp in wo_tiles(gi):
            cp.wait()
        for hd0 in WO_GROUPS[gi]:
            for half in range(2):
                hd = half * 16 + hd0
                acc = acc + jnp.dot(oa[:, hd * DH:(hd + 1) * DH],
                                    wo_v[hd * DH:(hd + 1) * DH, :],
                                    preferred_element_type=F32)
    a_out = acc.astype(BF16).astype(F32)
    r0 = g0 * a_out[0:1, :] + t0
    r1 = g1 * a_out[8:9, :] + t1
    o_ref[...] = jnp.concatenate([r0, r1], axis=0).astype(o_ref.dtype)


@jax.jit
def pallas_gated_mix__mha_block_cached__compressed_kv_cla__decode_kernel(
    A_x: jax.Array,
    A_k_cache: jax.Array,
    A_v_cache: jax.Array,
    A_wq: jax.Array,
    A_wo: jax.Array,
    B_x: jax.Array,
    B_c_kv: jax.Array,
    B_w_q: jax.Array,
    B_w_uk: jax.Array,
    B_w_uv: jax.Array,
    B_w_o: jax.Array,
    gate_w: jax.Array,
):
    del B_x
    k2 = A_k_cache.reshape(NBH * SK, DH)
    v2 = A_v_cache.reshape(NBH * SK, DH)
    ckv2 = B_c_kv.reshape(NB * SK, DM)
    bwq2 = B_w_q.reshape(DM * NH, DH)
    wuk2 = B_w_uk.reshape(DM * NH, DH)
    wuv2 = B_w_uv.reshape(DM * NH, DH)
    bwo2 = B_w_o.reshape(NH * DH, DM)

    any_spec = pl.BlockSpec(memory_space=pl.ANY)
    scratch = [
        pltpu.VMEM((NB, DM), BF16),
        pltpu.VMEM((DM,), BF16),
        pltpu.VMEM((NSLOT, SK, DH), BF16),
        pltpu.VMEM((NSLOT, SK, DH), BF16),
        pltpu.VMEM((DM, NH * DH), BF16),
        pltpu.VMEM((NH * DH, DM), BF16),
        pltpu.VMEM((NB * SK, DM), BF16),
        pltpu.VMEM((DM * NH, DH), BF16),
        pltpu.VMEM((DM * NH, DH), BF16),
        pltpu.VMEM((DM * NH, DH), BF16),
        pltpu.VMEM((NH * DH, DM), BF16),
        pltpu.VMEM((DM * NH // 2 + 16, DH), jnp.uint32),
        pltpu.VMEM((DM * NH // 2 + 16, DH), jnp.uint32),
        pltpu.VMEM((NB, 16, NH * DH), BF16),
        pltpu.VMEM((NB, 8, NH * DH), F32),
        pltpu.VMEM((NB, NH, DM), F32),
        pltpu.VMEM((NB, NH, SK), F32),
        pltpu.VMEM((NB, NH, 128), F32),
        pltpu.VMEM((NB, NH, 128), F32),
        pltpu.VMEM((NB, NH, DM), F32),
        pltpu.VMEM((16, DM), F32),
        pltpu.SemaphoreType.DMA((NGRP,)),
        pltpu.SemaphoreType.DMA((NGRP,)),
        pltpu.SemaphoreType.DMA((5,)),
    ]
    out = pl.pallas_call(
        _kernel,
        out_shape=jax.ShapeDtypeStruct((NB, DM), BF16),
        in_specs=[any_spec] * 11,
        out_specs=pl.BlockSpec(memory_space=pltpu.VMEM),
        scratch_shapes=scratch,
        compiler_params=pltpu.CompilerParams(vmem_limit_bytes=100 * 1024 * 1024),
    )(A_x.reshape(NB, DM), gate_w, k2, v2, A_wq, A_wo, ckv2, bwq2, wuk2, wuv2, bwo2)
    return out.reshape(NB, 1, DM)
```
